```python
import jax
import jax.numpy as jnp

def _softmax(x, axis=-1):
    return jax.nn.softmax(x, axis=axis)
def _gelu(x):
    return jax.nn.gelu(x, approximate=True)
def _silu(x):
    return jax.nn.silu(x)
def _sigmoid(x):
    return jax.nn.sigmoid(x)
def _layernorm(x, axis=-1, eps=1e-5):
    m = jnp.mean(x, axis=axis, keepdims=True)
    v = jnp.var(x, axis=axis, keepdims=True)
    return (x - m) / jnp.sqrt(v + eps)
def _scatter_add(tgt, idx, src, axis=0):
    return tgt.at[idx].add(src)
def _segment_sum(src, seg, n):
    return jax.ops.segment_sum(src, seg, n)
class _Rng:
    def __init__(self, key):
        self._k = key
    def _next(self):
        self._k, sub = jax.random.split(self._k)
        return sub
    def normal(self, shape):
        return jax.random.normal(self._next(), shape, dtype=jnp.bfloat16)
    def randint(self, lo, hi, shape):
        return jax.random.randint(self._next(), shape, lo, hi, dtype=jnp.int32)
    def uniform(self, shape, lo=0.0, hi=1.0):
        return jax.random.uniform(self._next(), shape, jnp.bfloat16, lo, hi)
    def permutation(self, n):
        return jax.random.permutation(self._next(), n)


kernel_name = 'parallel_sum__sliding_local_dilated__mixer_token_mlp__prompt'

def setup_inputs():
    _rng = _Rng(jax.random.key(int.from_bytes(__import__("os").urandom(4), "little")))
    _w = (lambda a: (lambda t: t.astype(jnp.bfloat16) if jnp.issubdtype(t.dtype, jnp.floating) else t)(jnp.asarray(a)))
    def _A_setup():
        B, S, D = 1, 2048, 448
        return {
            "x": _w((lambda *s: _rng.normal(s) * 0.05)(B, S, D)),
            "wqkv": _w((lambda *s: _rng.normal(s) * 0.05)(D, 3 * D)),
            "wo": _w((lambda *s: _rng.normal(s) * 0.05)(D, D)),
        }
    _A_in = _A_setup()

    def _B_setup():
        B, S, D, F = 1, 2048, 448, 1792
        return {
            "x": _w((lambda *s: _rng.normal(s) * 0.05)(B, S, D)),
            "w1": _w((lambda *s: _rng.normal(s) * 0.05)(S, F) * (S ** -0.5)),
            "b1": _w((lambda *s: _rng.normal(s) * 0.05)(F) * 0.02),
            "w2": _w((lambda *s: _rng.normal(s) * 0.05)(F, S) * (F ** -0.5)),
            "b2": _w((lambda *s: _rng.normal(s) * 0.05)(S) * 0.02),
        }
    _B_in = _B_setup()

    return {
        "A_x": _A_in["x"],
        "A_wqkv": _A_in["wqkv"],
        "A_wo": _A_in["wo"],
        "B_x": _B_in["x"],
        "B_w1": _B_in["w1"],
        "B_b1": _B_in["b1"],
        "B_w2": _B_in["w2"],
        "B_b2": _B_in["b2"],
    }

def reference(A_x, A_wqkv, A_wo, B_x, B_w1, B_b1, B_w2, B_b2):
    def _A_ref(x, wqkv, wo):
        B, S, D = x.shape
        H = 16; Dh = D // H
        W, dil = 8, 2
        qkv = (lambda x, *d: x.transpose(*d))((x @ wqkv).reshape(B, S, 3, H, Dh), 2, 0, 3, 1, 4)
        q, k, v = qkv[0], qkv[1], qkv[2]
        scale = Dh ** -0.5
        pos = jnp.arange(S)
        off = jnp.arange(W) * dil
        idx = pos[:, None] - off[None, :]
        mask = idx >= 0
        idx_c = jnp.where(mask, idx, 0).reshape(-1)
        kg = k[:, :, idx_c, :].reshape(B, H, S, W, Dh)
        vg = v[:, :, idx_c, :].reshape(B, H, S, W, Dh)
        logits = jnp.einsum("bhsd,bhswd->bhsw", q, kg) * scale
        logits = jnp.where(mask[None, None, :, :], logits, -1e9)
        attn = _softmax(logits, axis=-1)
        o = jnp.einsum("bhsw,bhswd->bhsd", attn, vg)
        return (lambda x, *d: x.transpose(*d))(o, 0, 2, 1, 3).reshape(B, S, D) @ wo

    def _B_ref(x, w1, b1, w2, b2):
        B, S, D = x.shape
        h = _layernorm(x, axis=-1)
        u = jnp.einsum("bsd,sf->bdf", h, w1) + b1
        u = _gelu(u)
        y = jnp.einsum("bdf,fs->bds", u, w2) + b2
        return (lambda x, *d: x.transpose(*d))(y, 0, 2, 1)

    x = A_x
    xn = _layernorm(x, axis=-1)
    return x + _A_ref(xn, A_wqkv, A_wo) + _B_ref(xn, B_w1, B_b1, B_w2, B_b2)
```

```python
import functools

import jax
import jax.numpy as jnp
import jax.experimental.pallas as pl
import jax.experimental.pallas.tpu as pltpu

S, D, F = 2048, 448, 1792
H, DH, W, DIL = 16, 28, 8, 2
TB = 256
FB = 256
NT = S // TB
NF = F // FB
PAD = 128

bf16 = jnp.bfloat16
f32 = jnp.float32


def _gelu(x):
    c = 0.7978845608028654
    return 0.5 * x * (1.0 + jnp.tanh(c * (x + 0.044715 * (x * x * x))))


def _kernel(x_hbm, wqkv_hbm, wo_hbm, w1_hbm, b1_ref, w2_hbm, b2_ref, out_hbm,
            x_v, wqkv_v, wo_v, w1_v, w2_v, xnT, wqkvT, woT, u_v, kT, vT, tmp, out_v,
            xsem, wsem, w1sem, w2sem, osem):
    def x_copy(i):
        return pltpu.make_async_copy(x_hbm.at[:, pl.ds(i * TB, TB)], x_v.at[:, pl.ds(i * TB, TB)], xsem.at[i])

    def w1_copy(i):
        return pltpu.make_async_copy(w1_hbm.at[:, pl.ds(i * FB, FB)], w1_v.at[i], w1sem.at[i])

    def w2_copy(i):
        return pltpu.make_async_copy(w2_hbm.at[:, pl.ds(i * TB, TB)], w2_v.at[i], w2sem.at[i])

    wqkv_copy = pltpu.make_async_copy(wqkv_hbm, wqkv_v, wsem.at[0])
    wo_copy = pltpu.make_async_copy(wo_hbm, wo_v, wsem.at[1])

    def out_copy(i):
        return pltpu.make_async_copy(out_v.at[i], out_hbm.at[:, pl.ds(i * TB, TB)], osem.at[i])

    x_copy(0).start()
    x_copy(1).start()

    def ln_body(i, c):
        x_copy(i).wait()

        @pl.when(i + 2 < NT)
        def _():
            x_copy(i + 2).start()

        @pl.when(i == NT - 2)
        def _():
            w1_copy(0).start()

        @pl.when(i == NT - 1)
        def _():
            wqkv_copy.start()
            wo_copy.start()

        r0 = pl.multiple_of(i * TB, TB)
        xt = x_v[:, pl.ds(r0, TB)].astype(f32)
        m = jnp.mean(xt, axis=0, keepdims=True)
        xc = xt - m
        v = jnp.mean(xc * xc, axis=0, keepdims=True)
        xnT[:, pl.ds(r0, TB)] = (xc * jax.lax.rsqrt(v + 1e-5)).astype(bf16)
        return c

    jax.lax.fori_loop(0, NT, ln_body, 0)

    kT[:, 0:PAD] = jnp.zeros((D, PAD), bf16)
    vT[:, 0:PAD] = jnp.zeros((D, PAD), bf16)

    wqkv_copy.wait()
    wt = wqkv_v[...].astype(f32).T
    for c in range(4):
        lo, hi = 128 * c, min(128 * (c + 1), D)
        tmp[c, :, 0:hi - lo] = wt[:, lo:hi]
    for t in range(3):
        for d in range(DH):
            rows = [tmp[c, pl.ds(t * D + d, H, stride=DH), :] for c in range(4)]
            blk = jnp.concatenate(rows, axis=1)[:, :D]
            wqkvT[pl.ds(t * D + d * H, H), :] = blk.astype(bf16)
    wo_copy.wait()
    wof = wo_v[...].astype(f32)
    for c in range(4):
        lo, hi = 128 * c, min(128 * (c + 1), D)
        tmp[c, 0:D, 0:hi - lo] = wof[:, lo:hi]
    blks = []
    for d in range(DH):
        rows = [tmp[c, pl.ds(d, H, stride=DH), :] for c in range(4)]
        blks.append(jnp.concatenate(rows, axis=1)[:, :D])
    woT[...] = jnp.concatenate(blks, axis=0).T.astype(bf16)

    def a_body(j, c):
        w1_copy(j).wait()

        @pl.when(j + 1 < NF)
        def _():
            w1_copy(j + 1).start()

        @pl.when(j + 1 == NF)
        def _():
            w2_copy(0).start()

        f0 = pl.multiple_of(j * FB, FB)
        u = jnp.dot(xnT[...], w1_v[j], preferred_element_type=f32)
        u = u + b1_ref[pl.ds(f0, FB)].astype(f32)[None, :]
        u_v[:, pl.ds(f0, FB)] = _gelu(u).astype(bf16)
        return c

    jax.lax.fori_loop(0, NF, a_body, 0)

    scale = DH ** -0.5

    def b_body(j, c):
        t0 = pl.multiple_of(j * TB, TB)
        w2_copy(j).wait()

        @pl.when(j + 1 < NT)
        def _():
            w2_copy(j + 1).start()

        qkv = jnp.dot(wqkvT[...], xnT[:, pl.ds(t0, TB)], preferred_element_type=f32)
        q = qkv[0:D]
        kT[:, pl.ds(t0 + PAD, TB)] = qkv[D:2 * D].astype(bf16)
        vT[:, pl.ds(t0 + PAD, TB)] = qkv[2 * D:3 * D].astype(bf16)
        y = jnp.dot(u_v[...], w2_v[j], preferred_element_type=f32)
        y = y + b2_ref[pl.ds(t0, TB)].astype(f32)[None, :]
        kw = kT[:, pl.ds(t0, TB + PAD)]
        vw = vT[:, pl.ds(t0, TB + PAD)]
        pos = t0 + jax.lax.broadcasted_iota(jnp.int32, (H, TB), 1)
        logits = []
        for w in range(W):
            ks = kw if w == 0 else pltpu.roll(kw, DIL * w, 1)
            ks = ks[:, PAD:].astype(f32)
            lg = (q * ks).reshape(DH, H, TB).sum(axis=0) * scale
            logits.append(jnp.where(pos >= DIL * w, lg, -1e9))
        mx = functools.reduce(jnp.maximum, logits)
        es = [jnp.exp(l - mx) for l in logits]
        den = functools.reduce(jnp.add, es)
        inv = 1.0 / den
        o = None
        for w in range(W):
            vs = vw if w == 0 else pltpu.roll(vw, DIL * w, 1)
            vs = vs[:, PAD:].astype(f32).reshape(DH, H, TB)
            term = vs * (es[w] * inv)[None]
            o = term if o is None else o + term
        oT = o.reshape(D, TB).astype(bf16)
        attnT = jnp.dot(woT[...], oT, preferred_element_type=f32)
        res = y + attnT + x_v[:, pl.ds(t0, TB)].astype(f32)
        out_v[j] = res.astype(bf16)
        out_copy(j).start()
        return c

    jax.lax.fori_loop(0, NT, b_body, 0)
    for i in range(NT):
        out_copy(i).wait()


@jax.jit
def pallas_parallel_sum__sliding_local_dilated__mixer_token_mlp__prompt_kernel(
    A_x: jax.Array,
    A_wqkv: jax.Array,
    A_wo: jax.Array,
    B_x: jax.Array,
    B_w1: jax.Array,
    B_b1: jax.Array,
    B_w2: jax.Array,
    B_b2: jax.Array,
):
    del B_x
    x = A_x.reshape(S, D).T
    any_spec = pl.BlockSpec(memory_space=pltpu.HBM)
    vmem_spec = pl.BlockSpec(memory_space=pltpu.VMEM)
    out = pl.pallas_call(
        _kernel,
        out_shape=jax.ShapeDtypeStruct((D, S), bf16),
        in_specs=[any_spec, any_spec, any_spec, any_spec, vmem_spec, any_spec, vmem_spec],
        out_specs=any_spec,
        scratch_shapes=[
            pltpu.VMEM((D, S), bf16),
            pltpu.VMEM((D, 3 * D), bf16),
            pltpu.VMEM((D, D), bf16),
            pltpu.VMEM((NF, S, FB), bf16),
            pltpu.VMEM((NT, F, TB), bf16),
            pltpu.VMEM((D, S), bf16),
            pltpu.VMEM((3 * D, D), bf16),
            pltpu.VMEM((D, D), bf16),
            pltpu.VMEM((D, F), bf16),
            pltpu.VMEM((D, S + PAD), bf16),
            pltpu.VMEM((D, S + PAD), bf16),
            pltpu.VMEM((4, 3 * D, 128), f32),
            pltpu.VMEM((NT, D, TB), bf16),
            pltpu.SemaphoreType.DMA((NT,)),
            pltpu.SemaphoreType.DMA((2,)),
            pltpu.SemaphoreType.DMA((NF,)),
            pltpu.SemaphoreType.DMA((NT,)),
            pltpu.SemaphoreType.DMA((NT,)),
        ],
        compiler_params=pltpu.CompilerParams(vmem_limit_bytes=100 * 1024 * 1024, disable_bounds_checks=True),
        name="fused_attn_mixer",
    )(x, A_wqkv, A_wo, B_w1, B_b1, B_w2, B_b2)
    return out.T.reshape(1, S, D)
```

```python
import functools


import jax
import jax.numpy as jnp
import jax.experimental.pallas as pl
import jax.experimental.pallas.tpu as pltpu

S, D, F = 2048, 448, 1792
H, DH, W, DIL = 16, 28, 8, 2
TB = 256
NT = S // TB
PAD = 128

bf16 = jnp.bfloat16
f32 = jnp.float32

SCOPES = True
ORDER = ["x0", "b1", "x1", "w1_0", "b2", "x2", "w1_1", "x3", "w1_2", "x4", "w1_3", "x5", "w1_4", "x6", "w1_5", "x7", "w1_6", "wqkv", "wo", "w1_7",
         ] + ["w2_%d" % i for i in range(NT)]
SEM = {"x%d" % i: i for i in range(NT)}
SEM.update({"w1_%d" % i: NT + i for i in range(NT)})
SEM.update({"w2_%d" % i: 2 * NT + i for i in range(NT)})
SEM.update({"wqkv": 3 * NT, "wo": 3 * NT + 1, "b1": 3 * NT + 2, "b2": 3 * NT + 3})


def _gelu(x):
    c = 0.7978845608028654
    return 0.5 * x * (1.0 + jnp.tanh(c * (x + 0.044715 * (x * x * x))))


def _scope(name):
    import contextlib
    return jax.named_scope(name) if SCOPES else contextlib.nullcontext()


def _kernel(x_hbm, wqkv_hbm, wo_hbm, w1_hbm, b1_hbm, w2_hbm, b2_hbm, out_hbm,
            b1_v, b2_v, x_v, wqkv_v, wo_v, w1_v, w2_v, xnT, wqkvT, woT, acc_v, u_v, kT, vT, tmp, tmp2, out_v,
            isem, osem):
    copies = {}
    for i in range(NT):
        copies["x%d" % i] = (x_hbm.at[:, pl.ds(i * TB, TB)], x_v.at[:, pl.ds(i * TB, TB)])
        copies["w1_%d" % i] = (w1_hbm.at[pl.ds(i * TB, TB), :], w1_v.at[pl.ds(i * TB, TB), :])
        copies["w2_%d" % i] = (w2_hbm.at[:, pl.ds(i * TB, TB)], w2_v.at[i])
    copies["wqkv"] = (wqkv_hbm, wqkv_v)
    copies["wo"] = (wo_hbm, wo_v)
    copies["b1"] = (b1_hbm, b1_v)
    copies["b2"] = (b2_hbm, b2_v)
    assert sorted(copies) == sorted(ORDER)
    dma = {n: pltpu.make_async_copy(copies[n][0], copies[n][1], isem.at[SEM[n]]) for n in ORDER}
    waited = set()

    def wait(*names):
        for n in names:
            if n not in waited:
                waited.add(n)
                dma[n].wait()

    def out_copy(i):
        return pltpu.make_async_copy(out_v.at[i], out_hbm.at[:, pl.ds(i * TB, TB)], osem.at[i])

    def prep_wqkv():
        wt = wqkv_v[...].astype(f32).T
        for c in range(4):
            lo, hi = 128 * c, min(128 * (c + 1), D)
            tmp[c, :, 0:hi - lo] = wt[:, lo:hi]
        for t in range(3):
            for d in range(DH):
                rows = [tmp[c, pl.ds(t * D + d, H, stride=DH), :] for c in range(4)]
                blk = jnp.concatenate(rows, axis=1)[:, :D]
                wqkvT[pl.ds(t * D + d * H, H), :] = blk.astype(bf16)

    def prep_wo():
        wof = wo_v[...].astype(f32)
        for c in range(4):
            lo, hi = 128 * c, min(128 * (c + 1), D)
            tmp2[c, :, 0:hi - lo] = wof[:, lo:hi]
        blks = []
        for d in range(DH):
            rows = [tmp2[c, pl.ds(d, H, stride=DH), :] for c in range(4)]
            blks.append(jnp.concatenate(rows, axis=1)[:, :D])
        woT[...] = jnp.concatenate(blks, axis=0).T.astype(bf16)
        kT[:, 0:PAD] = jnp.zeros((D, PAD), bf16)
        vT[:, 0:PAD] = jnp.zeros((D, PAD), bf16)

    def ds(i):
        if isinstance(i, int):
            return slice(i * TB, (i + 1) * TB)
        return pl.ds(pl.multiple_of(i * TB, TB), TB)

    def ln(i):
        xt = x_v[:, ds(i)].astype(f32)
        m = jnp.mean(xt, axis=0, keepdims=True)
        xc = xt - m
        v = jnp.mean(xc * xc, axis=0, keepdims=True)
        xnT[:, ds(i)] = (xc * jax.lax.rsqrt(v + 1e-5)).astype(bf16)

    def sweep(i, last):
        part = jnp.dot(xnT[:, ds(i)], w1_v[ds(i), :], preferred_element_type=f32)
        if not last:
            acc_v[...] = acc_v[...] + part
        else:
            u_v[...] = _gelu(acc_v[...] + part).astype(bf16)

    def x_dma(i):
        return pltpu.make_async_copy(x_hbm.at[:, ds(i)], x_v.at[:, ds(i)], isem.at[i])

    def w1_dma(i):
        return pltpu.make_async_copy(w1_hbm.at[ds(i), :], w1_v.at[ds(i), :], isem.at[NT + i])

    scale = DH ** -0.5

    def qkv_mm(j):
        t0 = j * TB
        qkv = jnp.dot(wqkvT[...], xnT[:, t0:t0 + TB], preferred_element_type=f32)
        kT[:, t0 + PAD:t0 + PAD + TB] = qkv[D:2 * D].astype(bf16)
        vT[:, t0 + PAD:t0 + PAD + TB] = qkv[2 * D:3 * D].astype(bf16)
        return qkv[0:D]

    def y_mm(j):
        t0 = j * TB
        y = jnp.dot(u_v[...], w2_v[j], preferred_element_type=f32)
        return y + b2_v[t0:t0 + TB].astype(f32)[None, :]

    def attn(j, q):
        t0 = j * TB
        kw = kT[:, t0:t0 + TB + PAD]
        vw = vT[:, t0:t0 + TB + PAD]
        pos = t0 + jax.lax.broadcasted_iota(jnp.int32, (H, TB), 1)
        logits = []
        for w in range(W):
            ks = kw if w == 0 else pltpu.roll(kw, DIL * w, 1)
            ks = ks[:, PAD:].astype(f32)
            lg = (q * ks).reshape(DH, H, TB).sum(axis=0) * scale
            logits.append(jnp.where(pos >= DIL * w, lg, -1e9) if t0 < DIL * w else lg)
        mx = functools.reduce(jnp.maximum, logits)
        es = [jnp.exp(l - mx) for l in logits]
        den = functools.reduce(jnp.add, es)
        inv = 1.0 / den
        o = None
        for w in range(W):
            vs = vw if w == 0 else pltpu.roll(vw, DIL * w, 1)
            vs = vs[:, PAD:].astype(f32).reshape(DH, H, TB)
            term = vs * (es[w] * inv)[None]
            o = term if o is None else o + term
        return o.reshape(D, TB).astype(bf16)

    def finish(j, y, oT):
        t0 = j * TB
        attnT = jnp.dot(woT[...], oT, preferred_element_type=f32)
        res = y + attnT + x_v[:, t0:t0 + TB].astype(f32)
        out_v[j] = res.astype(bf16)
        out_copy(j).start()

    for n in ORDER:
        dma[n].start()
    with _scope("p0"):
        wait("x0")
        ln(0)
        wait("b1")
        acc_v[...] = jnp.broadcast_to(b1_v[...].astype(f32)[None, :], (D, F))

    def sweep_body(i, c):
        w1_dma(i).wait()
        x_dma(i + 1).wait()
        sweep(i, False)
        ln(i + 1)
        return c

    with _scope("sweep"):
        jax.lax.fori_loop(0, NT - 1, sweep_body, 0)
    for i in range(NT - 1):
        waited.add("w1_%d" % i)
        waited.add("x%d" % (i + 1))
    with _scope("s7_wait"):
        wait("w1_7", "wqkv", "wo", "b2")
    with _scope("s7"):
        sweep(NT - 1, True)
        prep_wqkv()
        prep_wo()
    with _scope("b_wait0"):
        wait("w2_0", "w2_1", "w2_2", "w2_3")
    with _scope("b0"):
        q = qkv_mm(0)
        for j in range(4):
            y = y_mm(j)
            oT = attn(j, q)
            q = qkv_mm(j + 1)
            finish(j, y, oT)
    with _scope("b_wait1"):
        wait("w2_4", "w2_5", "w2_6", "w2_7")
    with _scope("b1"):
        for j in range(4, NT):
            y = y_mm(j)
            oT = attn(j, q)
            if j + 1 < NT:
                q = qkv_mm(j + 1)
            finish(j, y, oT)
    with _scope("end_wait"):
        for i in range(NT):
            out_copy(i).wait()
    assert waited == set(ORDER)


@jax.jit
def pallas_parallel_sum__sliding_local_dilated__mixer_token_mlp__prompt_kernel(
    A_x: jax.Array,
    A_wqkv: jax.Array,
    A_wo: jax.Array,
    B_x: jax.Array,
    B_w1: jax.Array,
    B_b1: jax.Array,
    B_w2: jax.Array,
    B_b2: jax.Array,
):
    del B_x
    x = A_x.reshape(S, D).T
    any_spec = pl.BlockSpec(memory_space=pltpu.HBM)
    out = pl.pallas_call(
        _kernel,
        out_shape=jax.ShapeDtypeStruct((D, S), bf16),
        in_specs=[any_spec] * 7,
        out_specs=any_spec,
        scratch_shapes=[
            pltpu.VMEM((F,), bf16),
            pltpu.VMEM((S,), bf16),
            pltpu.VMEM((D, S), bf16),
            pltpu.VMEM((D, 3 * D), bf16),
            pltpu.VMEM((D, D), bf16),
            pltpu.VMEM((S, F), bf16),
            pltpu.VMEM((NT, F, TB), bf16),
            pltpu.VMEM((D, S), bf16),
            pltpu.VMEM((3 * D, D), bf16),
            pltpu.VMEM((D, D), bf16),
            pltpu.VMEM((D, F), f32),
            pltpu.VMEM((D, F), bf16),
            pltpu.VMEM((D, S + PAD), bf16),
            pltpu.VMEM((D, S + PAD), bf16),
            pltpu.VMEM((4, 3 * D, 128), f32),
            pltpu.VMEM((4, D, 128), f32),
            pltpu.VMEM((NT, D, TB), bf16),
            pltpu.SemaphoreType.DMA((len(ORDER),)),
            pltpu.SemaphoreType.DMA((NT,)),
        ],
        compiler_params=pltpu.CompilerParams(vmem_limit_bytes=100 * 1024 * 1024, disable_bounds_checks=True),
        name="fused_attn_mixer",
    )(x, A_wqkv, A_wo, B_w1, B_b1, B_w2, B_b2)
    return out.T.reshape(1, S, D)
```

```python
import contextlib
import functools

import jax
import jax.numpy as jnp
import jax.experimental.pallas as pl
import jax.experimental.pallas.tpu as pltpu

S, D, F = 2048, 448, 1792
H, DH, W, DIL = 16, 28, 8, 2
TB = 256
NT = S // TB
PAD = 128
F0 = 768

bf16 = jnp.bfloat16
f32 = jnp.float32
u32 = jnp.uint32

SCOPES = True
SWEEP = [(1,), (2,), (3,), (4, 5), (6, 7)]
ORDER = ["x0", "b1", "w1_0a", "w1_0b", "x1", "w1_1", "x2", "w1_2", "x3", "w1_3", "x4", "x5", "w1_4", "w1_5", "x6", "x7",
         "w1_6", "wqkv", "w1_7", "wo", "b2"] + ["w2_%d" % i for i in range(NT)]
SEM = {n: k for k, n in enumerate(ORDER)}
W2SEM = SEM["w2_0"]


def _gelu(x):
    c = 0.7978845608028654
    return 0.5 * x * (1.0 + jnp.tanh(c * (x + 0.044715 * (x * x * x))))


def _pack(v):
    return pltpu.bitcast(v, u32)


def _unpack(v):
    return pltpu.bitcast(v, bf16)


def _scope(name):
    return jax.named_scope(name) if SCOPES else contextlib.nullcontext()


def _kernel(x_hbm, wqkv_hbm, wo_hbm, w1_hbm, b1_hbm, w2_hbm, b2_hbm, out_hbm,
            b1_v, b2_v, x_v, wqkv_v, wo_v, w1_v, w2_v, xnT, wqkvT, woT, acc_v, u_v, kT, vT, tmp, tmp2, out_v,
            isem, osem):
    copies = {}
    for i in range(NT):
        copies["x%d" % i] = (x_hbm.at[:, pl.ds(i * TB, TB)], x_v.at[:, pl.ds(i * TB, TB)])
        if i > 0:
            copies["w1_%d" % i] = (w1_hbm.at[pl.ds(i * TB, TB), :], w1_v.at[pl.ds(i * TB, TB), :])
        copies["w2_%d" % i] = (w2_hbm.at[:, pl.ds(i * TB, TB)], w2_v.at[i])
    copies["w1_0a"] = (w1_hbm.at[pl.ds(0, TB), pl.ds(0, F0)], w1_v.at[pl.ds(0, TB), pl.ds(0, F0)])
    copies["w1_0b"] = (w1_hbm.at[pl.ds(0, TB), pl.ds(F0, F - F0)], w1_v.at[pl.ds(0, TB), pl.ds(F0, F - F0)])
    copies["wqkv"] = (wqkv_hbm, wqkv_v)
    copies["wo"] = (wo_hbm, wo_v)
    copies["b1"] = (b1_hbm, b1_v)
    copies["b2"] = (b2_hbm, b2_v)
    assert sorted(copies) == sorted(ORDER)
    dma = {n: pltpu.make_async_copy(copies[n][0], copies[n][1], isem.at[SEM[n]]) for n in ORDER}
    waited = set()

    def wait(*names):
        for n in names:
            if n not in waited:
                waited.add(n)
                dma[n].wait()

    def ds(i, n=1, off=0):
        if isinstance(i, int):
            return slice(i * TB + off, (i + n) * TB + off)
        return pl.ds(pl.multiple_of(i * TB + off, 128), n * TB)

    def w2_dma(j):
        return pltpu.make_async_copy(w2_hbm.at[:, ds(j)], w2_v.at[j], isem.at[W2SEM + j])

    def out_copy(j):
        return pltpu.make_async_copy(out_v.at[j], out_hbm.at[:, ds(j)], osem.at[j])

    def ln(i):
        xt = x_v[:, ds(i)].astype(f32)
        m = jnp.mean(xt, axis=0, keepdims=True)
        xc = xt - m
        v = jnp.mean(xc * xc, axis=0, keepdims=True)
        xnT[:, ds(i)] = _pack((xc * jax.lax.rsqrt(v + 1e-5)).astype(bf16))

    def prep_wqkv():
        wt = wqkv_v[...].astype(f32).T
        for c in range(4):
            lo, hi = 128 * c, min(128 * (c + 1), D)
            tmp[c, :, 0:hi - lo] = wt[:, lo:hi]
        for t in range(3):
            for d in range(DH):
                rows = [tmp[c, pl.ds(t * D + d, H, stride=DH), :] for c in range(4)]
                blk = jnp.concatenate(rows, axis=1)[:, :D]
                wqkvT[pl.ds((t * D + d * H) // 2, H // 2), :] = _pack(blk.astype(bf16))

    def prep_wo():
        wof = wo_v[...].astype(f32)
        for c in range(4):
            lo, hi = 128 * c, min(128 * (c + 1), D)
            tmp2[c, :, 0:hi - lo] = wof[:, lo:hi]
        blks = []
        for d in range(DH):
            rows = [tmp2[c, pl.ds(d, H, stride=DH), :] for c in range(4)]
            blks.append(jnp.concatenate(rows, axis=1)[:, :D])
        woT[...] = _pack(jnp.concatenate(blks, axis=0).T.astype(bf16))
        kT[:, 0:PAD] = jnp.zeros((D // 2, PAD), u32)
        vT[:, 0:PAD] = jnp.zeros((D // 2, PAD), u32)

    def sweep_first(c0, c1):
        part = jnp.dot(_unpack(xnT[:, 0:TB]), w1_v[0:TB, c0:c1], preferred_element_type=f32)
        acc_v[:, c0:c1] = part + b1_v[c0:c1].astype(f32)[None, :]

    def sweep(blocks, last):
        k0, k1 = blocks[0] * TB, (blocks[-1] + 1) * TB
        part = jnp.dot(_unpack(xnT[:, k0:k1]), w1_v[k0:k1, :], preferred_element_type=f32)
        if not last:
            acc_v[...] = acc_v[...] + part
        else:
            u_v[...] = _pack(_gelu(acc_v[...] + part).astype(bf16))

    scale = DH ** -0.5

    def qkv_mm(j):
        qkv = jnp.dot(_unpack(wqkvT[...]), _unpack(xnT[:, ds(j)]), preferred_element_type=f32)
        kT[:, ds(j, 1, PAD)] = _pack(qkv[D:2 * D].astype(bf16))
        vT[:, ds(j, 1, PAD)] = _pack(qkv[2 * D:3 * D].astype(bf16))
        return qkv[0:D]

    def y_mm(j):
        y = jnp.dot(_unpack(u_v[...]), w2_v[j], preferred_element_type=f32)
        return y + b2_v[ds(j)].astype(f32)[None, :]

    def window(j):
        if isinstance(j, int):
            return slice(j * TB, (j + 1) * TB + PAD)
        return pl.ds(pl.multiple_of(j * TB, 128), TB + PAD)

    def attn(j, q, first):
        kw = kT[:, window(j)]
        vw = vT[:, window(j)]
        pos = jax.lax.broadcasted_iota(jnp.int32, (H, TB), 1)
        logits = []
        for w in range(W):
            ks = kw if w == 0 else pltpu.roll(kw, DIL * w, 1)
            ks = _unpack(ks[:, PAD:]).astype(f32)
            lg = (q * ks).reshape(DH, H, TB).sum(axis=0) * scale
            logits.append(jnp.where(pos >= DIL * w, lg, -1e9) if first else lg)
        mx = functools.reduce(jnp.maximum, logits)
        es = [jnp.exp(l - mx) for l in logits]
        den = functools.reduce(jnp.add, es)
        inv = 1.0 / den
        o = None
        for w in range(W):
            vs = vw if w == 0 else pltpu.roll(vw, DIL * w, 1)
            vs = _unpack(vs[:, PAD:]).astype(f32).reshape(DH, H, TB)
            term = vs * (es[w] * inv)[None]
            o = term if o is None else o + term
        return o.reshape(D, TB).astype(bf16)

    def finish(j, y, oT):
        attnT = jnp.dot(_unpack(woT[...]), oT, preferred_element_type=f32)
        res = y + attnT + x_v[:, ds(j)].astype(f32)
        out_v[j] = res.astype(bf16)
        out_copy(j).start()

    for n in ORDER:
        dma[n].start()
    with _scope("p0"):
        wait("x0")
        ln(0)
    with _scope("s0a_wait"):
        wait("b1", "w1_0a")
    with _scope("s0a"):
        sweep_first(0, F0)
    with _scope("s0b_wait"):
        wait("w1_0b", "x1")
    with _scope("s0b"):
        sweep_first(F0, F)
        ln(1)
    nsw = len(SWEEP)
    for r in range(nsw):
        nxt = SWEEP[r + 1] if r + 1 < nsw else ()
        with _scope("s%d_wait" % (r + 1)):
            wait(*["w1_%d" % b for b in SWEEP[r]], *["x%d" % b for b in nxt])
            if r == nsw - 1:
                wait("wqkv", "wo")
        with _scope("s%d" % (r + 1)):
            sweep(SWEEP[r], r == nsw - 1)
            for b in nxt:
                ln(b)
            if r == nsw - 1:
                prep_wqkv()
                prep_wo()
                q = qkv_mm(0)

    GROUP = 3

    def b_body(i, q):
        j0 = i * GROUP
        for jj in range(GROUP):
            w2_dma(j0 + jj).wait()
        for jj in range(GROUP):
            j = j0 + jj
            y = y_mm(j)
            oT = attn(j, q, jj == 0)[...] if False else attn_dyn(i, j, jj, q)
            q = qkv_mm(j + 1)
            finish(j, y, oT)
        return q

    def attn_dyn(i, j, jj, q):
        if jj != 0:
            return attn(j, q, False)
        return attn_masked(i, j, q)

    def attn_masked(i, j, q):
        kw = kT[:, window(j)]
        vw = vT[:, window(j)]
        pos = jax.lax.broadcasted_iota(jnp.int32, (H, TB), 1) + j * TB
        logits = []
        for w in range(W):
            ks = kw if w == 0 else pltpu.roll(kw, DIL * w, 1)
            ks = _unpack(ks[:, PAD:]).astype(f32)
            lg = (q * ks).reshape(DH, H, TB).sum(axis=0) * scale
            logits.append(jnp.where(pos >= DIL * w, lg, -1e9) if w else lg)
        mx = functools.reduce(jnp.maximum, logits)
        es = [jnp.exp(l - mx) for l in logits]
        inv = 1.0 / functools.reduce(jnp.add, es)
        o = None
        for w in range(W):
            vs = vw if w == 0 else pltpu.roll(vw, DIL * w, 1)
            vs = _unpack(vs[:, PAD:]).astype(f32).reshape(DH, H, TB)
            term = vs * (es[w] * inv)[None]
            o = term if o is None else o + term
        return o.reshape(D, TB).astype(bf16)

    with _scope("b_loop"):
        wait("b2")
        q = jax.lax.fori_loop(0, 2, b_body, q)
    for j in range(2 * GROUP):
        waited.add("w2_%d" % j)
    with _scope("b_tail_wait"):
        wait("w2_6", "w2_7")
    with _scope("b_tail"):
        for j in range(2 * GROUP, NT):
            y = y_mm(j)
            oT = attn(j, q, False)
            if j + 1 < NT:
                q = qkv_mm(j + 1)
            finish(j, y, oT)
    with _scope("end_wait"):
        for i in range(NT):
            out_copy(i).wait()
    assert waited == set(ORDER), set(ORDER) - waited


@jax.jit
def pallas_parallel_sum__sliding_local_dilated__mixer_token_mlp__prompt_kernel(
    A_x: jax.Array,
    A_wqkv: jax.Array,
    A_wo: jax.Array,
    B_x: jax.Array,
    B_w1: jax.Array,
    B_b1: jax.Array,
    B_w2: jax.Array,
    B_b2: jax.Array,
):
    del B_x
    x = A_x.reshape(S, D).T
    any_spec = pl.BlockSpec(memory_space=pltpu.HBM)
    out = pl.pallas_call(
        _kernel,
        out_shape=jax.ShapeDtypeStruct((D, S), bf16),
        in_specs=[any_spec] * 7,
        out_specs=any_spec,
        scratch_shapes=[
            pltpu.VMEM((F,), bf16),
            pltpu.VMEM((S,), bf16),
            pltpu.VMEM((D, S), bf16),
            pltpu.VMEM((D, 3 * D), bf16),
            pltpu.VMEM((D, D), bf16),
            pltpu.VMEM((S, F), bf16),
            pltpu.VMEM((NT, F, TB), bf16),
            pltpu.VMEM((D // 2, S), u32),
            pltpu.VMEM((3 * D // 2, D), u32),
            pltpu.VMEM((D // 2, D), u32),
            pltpu.VMEM((D, F), f32),
            pltpu.VMEM((D // 2, F), u32),
            pltpu.VMEM((D // 2, S + PAD), u32),
            pltpu.VMEM((D // 2, S + PAD), u32),
            pltpu.VMEM((4, 3 * D, 128), f32),
            pltpu.VMEM((4, D, 128), f32),
            pltpu.VMEM((NT, D, TB), bf16),
            pltpu.SemaphoreType.DMA((len(ORDER),)),
            pltpu.SemaphoreType.DMA((NT,)),
        ],
        compiler_params=pltpu.CompilerParams(vmem_limit_bytes=100 * 1024 * 1024, disable_bounds_checks=True,
                                             disable_semaphore_checks=True),
        name="fused_attn_mixer",
    )(x, A_wqkv, A_wo, B_w1, B_b1, B_w2, B_b2)
    return out.T.reshape(1, S, D)
```

```python
import contextlib
import functools

import jax
import jax.numpy as jnp
import jax.experimental.pallas as pl
import jax.experimental.pallas.tpu as pltpu

S, D, F = 2048, 448, 1792
H, DH, W, DIL = 16, 28, 8, 2
TB = 256
NT = S // TB
PAD = 128
F0 = 768

bf16 = jnp.bfloat16
f32 = jnp.float32
u32 = jnp.uint32

SCOPES = True
SWEEP = [(1,), (2,), (3,), (4, 5), (6, 7)]
ORDER = ["x0", "b1", "w1_0a", "w1_0b", "x1", "w1_1", "x2", "w1_2", "x3", "w1_3", "x4", "w1_4", "x5", "w1_5", "x6", "w1_6", "x7",
         "wqkv", "w1_7", "wo", "b2"] + ["w2_%d" % i for i in range(NT)]
SEM = {"x%d" % i: i for i in range(NT)}
SEM.update({"w1_%d" % i: NT + i for i in range(1, NT)})
SEM.update({"w2_%d" % i: 2 * NT + i for i in range(NT)})
SEM.update({"w1_0a": NT, "w1_0b": 3 * NT, "wqkv": 3 * NT + 1, "wo": 3 * NT + 2, "b1": 3 * NT + 3, "b2": 3 * NT + 4})


def _gelu(x):
    c = 0.7978845608028654
    return 0.5 * x * (1.0 + jnp.tanh(c * (x + 0.044715 * (x * x * x))))


def _pack(v):
    return pltpu.bitcast(v, u32)


def _unpack(v):
    return pltpu.bitcast(v, bf16)


def _scope(name):
    return jax.named_scope(name) if SCOPES else contextlib.nullcontext()


def _kernel(x_hbm, wqkv_hbm, wo_hbm, w1_hbm, b1_hbm, w2_hbm, b2_hbm, out_hbm,
            b1_v, b2_v, x_v, wqkv_v, wo_v, w1_v, w2_v, xnT, wqkvT, woT, acc_v, u_v, kT, vT, tmp, tmp2, out_v,
            isem, osem):
    copies = {}
    for i in range(NT):
        copies["x%d" % i] = (x_hbm.at[:, pl.ds(i * TB, TB)], x_v.at[:, pl.ds(i * TB, TB)])
        if i > 0:
            copies["w1_%d" % i] = (w1_hbm.at[pl.ds(i * TB, TB), :], w1_v.at[pl.ds(i * TB, TB), :])
        copies["w2_%d" % i] = (w2_hbm.at[:, pl.ds(i * TB, TB)], w2_v.at[i])
    copies["w1_0a"] = (w1_hbm.at[pl.ds(0, TB), pl.ds(0, F0)], w1_v.at[pl.ds(0, TB), pl.ds(0, F0)])
    copies["w1_0b"] = (w1_hbm.at[pl.ds(0, TB), pl.ds(F0, F - F0)], w1_v.at[pl.ds(0, TB), pl.ds(F0, F - F0)])
    copies["wqkv"] = (wqkv_hbm, wqkv_v)
    copies["wo"] = (wo_hbm, wo_v)
    copies["b1"] = (b1_hbm, b1_v)
    copies["b2"] = (b2_hbm, b2_v)
    assert sorted(copies) == sorted(ORDER)
    dma = {n: pltpu.make_async_copy(copies[n][0], copies[n][1], isem.at[SEM[n]]) for n in ORDER}
    waited = set()

    def wait(*names):
        for n in names:
            if n not in waited:
                waited.add(n)
                dma[n].wait()

    def ds(i, n=1, off=0):
        if isinstance(i, int):
            return slice(i * TB + off, (i + n) * TB + off)
        return pl.ds(pl.multiple_of(i * TB + off, 128), n * TB)

    def w2_dma(j):
        return pltpu.make_async_copy(w2_hbm.at[:, ds(j)], w2_v.at[j], isem.at[W2SEM + j])

    def out_copy(j):
        return pltpu.make_async_copy(out_v.at[j], out_hbm.at[:, ds(j)], osem.at[j])

    def ln(i):
        xt = x_v[:, ds(i)].astype(f32)
        m = jnp.mean(xt, axis=0, keepdims=True)
        xc = xt - m
        v = jnp.mean(xc * xc, axis=0, keepdims=True)
        xnT[:, ds(i)] = _pack((xc * jax.lax.rsqrt(v + 1e-5)).astype(bf16))

    def prep_wqkv():
        wt = wqkv_v[...].astype(f32).T
        for c in range(4):
            lo, hi = 128 * c, min(128 * (c + 1), D)
            tmp[c, :, 0:hi - lo] = wt[:, lo:hi]
        for t in range(3):
            for d in range(DH):
                rows = [tmp[c, pl.ds(t * D + d, H, stride=DH), :] for c in range(4)]
                blk = jnp.concatenate(rows, axis=1)[:, :D]
                wqkvT[pl.ds((t * D + d * H) // 2, H // 2), :] = _pack(blk.astype(bf16))

    def prep_wo():
        wof = wo_v[...].astype(f32)
        for c in range(4):
            lo, hi = 128 * c, min(128 * (c + 1), D)
            tmp2[c, :, 0:hi - lo] = wof[:, lo:hi]
        blks = []
        for d in range(DH):
            rows = [tmp2[c, pl.ds(d, H, stride=DH), :] for c in range(4)]
            blks.append(jnp.concatenate(rows, axis=1)[:, :D])
        woT[...] = _pack(jnp.concatenate(blks, axis=0).T.astype(bf16))
        kT[:, 0:PAD] = jnp.zeros((D // 2, PAD), u32)
        vT[:, 0:PAD] = jnp.zeros((D // 2, PAD), u32)

    def sweep_first(c0, c1):
        part = jnp.dot(_unpack(xnT[:, 0:TB]), w1_v[0:TB, c0:c1], preferred_element_type=f32)
        acc_v[:, c0:c1] = part + b1_v[c0:c1].astype(f32)[None, :]

    def sweep(blocks, last):
        k0, k1 = blocks[0] * TB, (blocks[-1] + 1) * TB
        part = jnp.dot(_unpack(xnT[:, k0:k1]), w1_v[k0:k1, :], preferred_element_type=f32)
        if not last:
            acc_v[...] = acc_v[...] + part
        else:
            u_v[...] = _pack(_gelu(acc_v[...] + part).astype(bf16))

    scale = DH ** -0.5

    def qkv_mm(j):
        qkv = jnp.dot(_unpack(wqkvT[...]), _unpack(xnT[:, ds(j)]), preferred_element_type=f32)
        kT[:, ds(j, 1, PAD)] = _pack(qkv[D:2 * D].astype(bf16))
        vT[:, ds(j, 1, PAD)] = _pack(qkv[2 * D:3 * D].astype(bf16))
        return qkv[0:D]

    def y_mm(j):
        y = jnp.dot(_unpack(u_v[...]), w2_v[j], preferred_element_type=f32)
        return y + b2_v[ds(j)].astype(f32)[None, :]

    def window(j):
        if isinstance(j, int):
            return slice(j * TB, (j + 1) * TB + PAD)
        return pl.ds(pl.multiple_of(j * TB, 128), TB + PAD)

    def attn(j, q, first):
        kw = kT[:, window(j)]
        vw = vT[:, window(j)]
        pos = jax.lax.broadcasted_iota(jnp.int32, (H, TB), 1)
        logits = []
        for w in range(W):
            ks = kw if w == 0 else pltpu.roll(kw, DIL * w, 1)
            ks = _unpack(ks[:, PAD:]).astype(f32)
            lg = (q * ks).reshape(DH, H, TB).sum(axis=0) * scale
            logits.append(jnp.where(pos >= DIL * w, lg, -1e9) if first else lg)
        mx = functools.reduce(jnp.maximum, logits)
        es = [jnp.exp(l - mx) for l in logits]
        den = functools.reduce(jnp.add, es)
        inv = 1.0 / den
        o = None
        for w in range(W):
            vs = vw if w == 0 else pltpu.roll(vw, DIL * w, 1)
            vs = _unpack(vs[:, PAD:]).astype(f32).reshape(DH, H, TB)
            term = vs * (es[w] * inv)[None]
            o = term if o is None else o + term
        return o.reshape(D, TB).astype(bf16)

    def finish(j, y, oT):
        attnT = jnp.dot(_unpack(woT[...]), oT, preferred_element_type=f32)
        res = y + attnT + x_v[:, ds(j)].astype(f32)
        out_v[j] = res.astype(bf16)
        out_copy(j).start()

    for n in ORDER:
        dma[n].start()
    with _scope("p0"):
        wait("x0")
        ln(0)
    with _scope("s0a_wait"):
        wait("b1", "w1_0a")
    with _scope("s0a"):
        sweep_first(0, F0)
    with _scope("s0b_wait"):
        wait("w1_0b", "x1")
    with _scope("s0b"):
        sweep_first(F0, F)
        ln(1)
    def sweep_body(i, c):
        pltpu.make_async_copy(w1_hbm.at[ds(i), :], w1_v.at[ds(i), :], isem.at[NT + i]).wait()
        pltpu.make_async_copy(x_hbm.at[:, ds(i + 1)], x_v.at[:, ds(i + 1)], isem.at[i + 1]).wait()
        part = jnp.dot(_unpack(xnT[:, ds(i)]), w1_v[ds(i), :], preferred_element_type=f32)
        acc_v[...] = acc_v[...] + part
        ln(i + 1)
        return c

    with _scope("sweep_loop"):
        jax.lax.fori_loop(1, 7, sweep_body, 0)
    for i in range(1, 7):
        waited.add("w1_%d" % i)
        waited.add("x%d" % (i + 1))
    with _scope("s5_wait"):
        wait("w1_7", "wqkv", "wo")
    with _scope("s5"):
        sweep((7,), True)
        prep_wqkv()
        prep_wo()
        q = qkv_mm(0)
    with _scope("b_wait0"):
        wait("b2", "w2_0", "w2_1", "w2_2", "w2_3")
    with _scope("b0"):
        for j in range(4):
            y = y_mm(j)
            oT = attn(j, q, j == 0)
            q = qkv_mm(j + 1)
            finish(j, y, oT)
    with _scope("b_wait1"):
        wait("w2_4", "w2_5", "w2_6", "w2_7")
    with _scope("b1"):
        for j in range(4, NT):
            y = y_mm(j)
            oT = attn(j, q, False)
            if j + 1 < NT:
                q = qkv_mm(j + 1)
            finish(j, y, oT)
    with _scope("end_wait"):
        for i in range(NT):
            out_copy(i).wait()
    assert waited == set(ORDER), set(ORDER) - waited


@jax.jit
def pallas_parallel_sum__sliding_local_dilated__mixer_token_mlp__prompt_kernel(
    A_x: jax.Array,
    A_wqkv: jax.Array,
    A_wo: jax.Array,
    B_x: jax.Array,
    B_w1: jax.Array,
    B_b1: jax.Array,
    B_w2: jax.Array,
    B_b2: jax.Array,
):
    del B_x
    x = A_x.reshape(S, D).T
    any_spec = pl.BlockSpec(memory_space=pltpu.HBM)
    out = pl.pallas_call(
        _kernel,
        out_shape=jax.ShapeDtypeStruct((D, S), bf16),
        in_specs=[any_spec] * 7,
        out_specs=any_spec,
        scratch_shapes=[
            pltpu.VMEM((F,), bf16),
            pltpu.VMEM((S,), bf16),
            pltpu.VMEM((D, S), bf16),
            pltpu.VMEM((D, 3 * D), bf16),
            pltpu.VMEM((D, D), bf16),
            pltpu.VMEM((S, F), bf16),
            pltpu.VMEM((NT, F, TB), bf16),
            pltpu.VMEM((D // 2, S), u32),
            pltpu.VMEM((3 * D // 2, D), u32),
            pltpu.VMEM((D // 2, D), u32),
            pltpu.VMEM((D, F), f32),
            pltpu.VMEM((D // 2, F), u32),
            pltpu.VMEM((D // 2, S + PAD), u32),
            pltpu.VMEM((D // 2, S + PAD), u32),
            pltpu.VMEM((4, 3 * D, 128), f32),
            pltpu.VMEM((4, D, 128), f32),
            pltpu.VMEM((NT, D, TB), bf16),
            pltpu.SemaphoreType.DMA((3 * NT + 5,)),
            pltpu.SemaphoreType.DMA((NT,)),
        ],
        compiler_params=pltpu.CompilerParams(vmem_limit_bytes=100 * 1024 * 1024, disable_bounds_checks=True,
                                             disable_semaphore_checks=True),
        name="fused_attn_mixer",
    )(x, A_wqkv, A_wo, B_w1, B_b1, B_w2, B_b2)
    return out.T.reshape(1, S, D)
```

```python
import contextlib
import functools

import jax
import jax.numpy as jnp
import jax.experimental.pallas as pl
import jax.experimental.pallas.tpu as pltpu

S, D, F = 2048, 448, 1792
H, DH, W, DIL = 16, 28, 8, 2
TB = 256
NT = S // TB
PAD = 128
F0 = 768

bf16 = jnp.bfloat16
f32 = jnp.float32
u32 = jnp.uint32

SCOPES = False
SWEEP = [(1,), (2,), (3,), (4, 5), (6, 7)]
ORDER = ["x0", "b1", "w1_0a", "w1_0b", "x1", "w1_1", "x2", "w1_2", "x3", "w1_3", "x4", "w1_4", "x5", "w1_5", "x6", "x7", "w1_6", "w1_7",
         "wqkv", "wo", "b2"] + ["w2_%d" % i for i in range(NT)]
SEM = {"x%d" % i: i for i in range(NT)}
SEM.update({"w1_%d" % i: NT + i for i in range(1, NT)})
SEM.update({"w2_%d" % i: 2 * NT + i for i in range(NT)})
SEM.update({"w1_0a": NT, "w1_0b": 3 * NT, "wqkv": 3 * NT + 1, "wo": 3 * NT + 2, "b1": 3 * NT + 3, "b2": 3 * NT + 4})


def _gelu(x):
    c = 0.7978845608028654
    return 0.5 * x * (1.0 + jnp.tanh(c * (x + 0.044715 * (x * x * x))))


def _pack(v):
    return pltpu.bitcast(v, u32)


def _unpack(v):
    return pltpu.bitcast(v, bf16)


def _scope(name):
    return jax.named_scope(name) if SCOPES else contextlib.nullcontext()


def _kernel(x_hbm, wqkv_hbm, wo_hbm, w1_hbm, b1_hbm, w2_hbm, b2_hbm, out_hbm,
            b1_v, b2_v, x_v, wqkv_v, wo_v, w1_v, w2_v, xnT, wqkvT, woT, acc_v, u_v, kT, vT, tmp, tmp2, out_v,
            isem, osem):
    copies = {}
    for i in range(NT):
        copies["x%d" % i] = (x_hbm.at[:, pl.ds(i * TB, TB)], x_v.at[:, pl.ds(i * TB, TB)])
        if i > 0:
            copies["w1_%d" % i] = (w1_hbm.at[pl.ds(i * TB, TB), :], w1_v.at[pl.ds(i * TB, TB), :])
        copies["w2_%d" % i] = (w2_hbm.at[:, pl.ds(i * TB, TB)], w2_v.at[i])
    copies["w1_0a"] = (w1_hbm.at[pl.ds(0, TB), pl.ds(0, F0)], w1_v.at[pl.ds(0, TB), pl.ds(0, F0)])
    copies["w1_0b"] = (w1_hbm.at[pl.ds(0, TB), pl.ds(F0, F - F0)], w1_v.at[pl.ds(0, TB), pl.ds(F0, F - F0)])
    copies["wqkv"] = (wqkv_hbm, wqkv_v)
    copies["wo"] = (wo_hbm, wo_v)
    copies["b1"] = (b1_hbm, b1_v)
    copies["b2"] = (b2_hbm, b2_v)
    assert sorted(copies) == sorted(ORDER)
    dma = {n: pltpu.make_async_copy(copies[n][0], copies[n][1], isem.at[SEM[n]]) for n in ORDER}
    waited = set()

    def wait(*names):
        for n in names:
            if n not in waited:
                waited.add(n)
                dma[n].wait()

    def ds(i, n=1, off=0):
        if isinstance(i, int):
            return slice(i * TB + off, (i + n) * TB + off)
        return pl.ds(pl.multiple_of(i * TB + off, 128), n * TB)

    def w2_dma(j):
        return pltpu.make_async_copy(w2_hbm.at[:, ds(j)], w2_v.at[j], isem.at[W2SEM + j])

    def out_copy(j):
        return pltpu.make_async_copy(out_v.at[j], out_hbm.at[:, ds(j)], osem.at[j])

    RL = D // 7
    last_copies = [pltpu.make_async_copy(out_v.at[NT - 1, pl.ds(p * RL, RL), :],
                                         out_hbm.at[pl.ds(p * RL, RL), pl.ds((NT - 1) * TB, TB)], osem.at[NT + p]) for p in range(7)]

    def ln(i):
        xt = x_v[:, ds(i)].astype(f32)
        m = jnp.mean(xt, axis=0, keepdims=True)
        xc = xt - m
        v = jnp.mean(xc * xc, axis=0, keepdims=True)
        xnT[:, ds(i)] = _pack((xc * jax.lax.rsqrt(v + 1e-5)).astype(bf16))

    def prep_wqkv():
        wt = wqkv_v[...].astype(f32).T
        for c in range(4):
            lo, hi = 128 * c, min(128 * (c + 1), D)
            tmp[c, :, 0:hi - lo] = wt[:, lo:hi]
        for t in range(3):
            for d in range(DH):
                rows = [tmp[c, pl.ds(t * D + d, H, stride=DH), :] for c in range(4)]
                blk = jnp.concatenate(rows, axis=1)[:, :D]
                wqkvT[pl.ds((t * D + d * H) // 2, H // 2), :] = _pack(blk.astype(bf16))

    def prep_wo():
        wof = wo_v[...].astype(f32)
        for c in range(4):
            lo, hi = 128 * c, min(128 * (c + 1), D)
            tmp2[c, :, 0:hi - lo] = wof[:, lo:hi]
        blks = []
        for d in range(DH):
            rows = [tmp2[c, pl.ds(d, H, stride=DH), :] for c in range(4)]
            blks.append(jnp.concatenate(rows, axis=1)[:, :D])
        woT[...] = _pack(jnp.concatenate(blks, axis=0).T.astype(bf16))
        kT[:, 0:PAD] = jnp.zeros((D // 2, PAD), u32)
        vT[:, 0:PAD] = jnp.zeros((D // 2, PAD), u32)

    def sweep_first(c0, c1):
        part = jnp.dot(_unpack(xnT[:, 0:TB]), w1_v[0:TB, c0:c1], preferred_element_type=f32)
        acc_v[:, c0:c1] = part + b1_v[c0:c1].astype(f32)[None, :]

    def sweep(blocks, last):
        k0, k1 = blocks[0] * TB, (blocks[-1] + 1) * TB
        part = jnp.dot(_unpack(xnT[:, k0:k1]), w1_v[k0:k1, :], preferred_element_type=f32)
        if not last:
            acc_v[...] = acc_v[...] + part
        else:
            u_v[...] = _pack(_gelu(acc_v[...] + part).astype(bf16))

    scale = DH ** -0.5

    def qkv_mm(j):
        qkv = jnp.dot(_unpack(wqkvT[...]), _unpack(xnT[:, ds(j)]), preferred_element_type=f32)
        kT[:, ds(j, 1, PAD)] = _pack(qkv[D:2 * D].astype(bf16))
        vT[:, ds(j, 1, PAD)] = _pack(qkv[2 * D:3 * D].astype(bf16))
        return qkv[0:D]

    def y_mm(j):
        y = jnp.dot(_unpack(u_v[...]), w2_v[j], preferred_element_type=f32)
        return y + b2_v[ds(j)].astype(f32)[None, :]

    def window(j):
        if isinstance(j, int):
            return slice(j * TB, (j + 1) * TB + PAD)
        return pl.ds(pl.multiple_of(j * TB, 128), TB + PAD)

    def attn(j, q, first):
        kw = kT[:, window(j)]
        vw = vT[:, window(j)]
        pos = jax.lax.broadcasted_iota(jnp.int32, (H, TB), 1)
        logits = []
        for w in range(W):
            ks = kw if w == 0 else pltpu.roll(kw, DIL * w, 1)
            ks = _unpack(ks[:, PAD:]).astype(f32)
            lg = (q * ks).reshape(DH, H, TB).sum(axis=0) * scale
            logits.append(jnp.where(pos >= DIL * w, lg, -1e9) if first else lg)
        mx = functools.reduce(jnp.maximum, logits)
        es = [jnp.exp(l - mx) for l in logits]
        den = functools.reduce(jnp.add, es)
        inv = 1.0 / den
        o = None
        for w in range(W):
            vs = vw if w == 0 else pltpu.roll(vw, DIL * w, 1)
            vs = _unpack(vs[:, PAD:]).astype(f32).reshape(DH, H, TB)
            term = vs * (es[w] * inv)[None]
            o = term if o is None else o + term
        return o.reshape(D, TB).astype(bf16)

    def finish_last(j, y, oT):
        attnT = jnp.dot(_unpack(woT[...]), oT, preferred_element_type=f32)
        res = y + attnT + x_v[:, ds(j)].astype(f32)
        R = D // 7
        for p in range(7):
            out_v[j, p * R:(p + 1) * R, :] = res[p * R:(p + 1) * R].astype(bf16)
            last_copies[p].start()

    def finish(j, y, oT):
        attnT = jnp.dot(_unpack(woT[...]), oT, preferred_element_type=f32)
        res = y + attnT + x_v[:, ds(j)].astype(f32)
        out_v[j] = res.astype(bf16)
        out_copy(j).start()

    for n in ORDER:
        dma[n].start()
    with _scope("p0"):
        wait("x0")
        ln(0)
    with _scope("s0a_wait"):
        wait("b1", "w1_0a")
    with _scope("s0a"):
        sweep_first(0, F0)
    with _scope("s0b_wait"):
        wait("w1_0b", "x1")
    with _scope("s0b"):
        sweep_first(F0, F)
        ln(1)
    def sweep_body(i, c):
        pltpu.make_async_copy(w1_hbm.at[ds(i), :], w1_v.at[ds(i), :], isem.at[NT + i]).wait()
        pltpu.make_async_copy(x_hbm.at[:, ds(i + 1)], x_v.at[:, ds(i + 1)], isem.at[i + 1]).wait()
        part = jnp.dot(_unpack(xnT[:, ds(i)]), w1_v[ds(i), :], preferred_element_type=f32)
        acc_v[...] = acc_v[...] + part
        ln(i + 1)
        return c

    with _scope("sweep_loop"):
        jax.lax.fori_loop(1, 6, sweep_body, 0)
    for i in range(1, 6):
        waited.add("w1_%d" % i)
        waited.add("x%d" % (i + 1))
    with _scope("s5_wait"):
        wait("x7", "w1_6", "w1_7", "wqkv", "wo")
    with _scope("s5"):
        p6 = jnp.dot(_unpack(xnT[:, ds(6)]), w1_v[ds(6), :], preferred_element_type=f32)
        ln(7)
        p7 = jnp.dot(_unpack(xnT[:, ds(7)]), w1_v[ds(7), :], preferred_element_type=f32)
        u_v[...] = _pack(_gelu(acc_v[...] + p6 + p7).astype(bf16))
        prep_wqkv()
        prep_wo()
        q = qkv_mm(0)
    with _scope("b_wait0"):
        wait("b2", "w2_0", "w2_1", "w2_2", "w2_3")
    with _scope("b0"):
        for j in range(4):
            y = y_mm(j)
            oT = attn(j, q, j == 0)
            q = qkv_mm(j + 1)
            finish(j, y, oT)
    with _scope("b_wait1"):
        wait("w2_4", "w2_5", "w2_6", "w2_7")
    with _scope("b1"):
        for j in range(4, NT):
            y = y_mm(j)
            oT = attn(j, q, False)
            if j + 1 < NT:
                q = qkv_mm(j + 1)
            (finish if j + 1 < NT else finish_last)(j, y, oT)
    with _scope("end_wait"):
        for i in range(NT - 1):
            out_copy(i).wait()
        for c in last_copies:
            c.wait()
    assert waited == set(ORDER), set(ORDER) - waited


@jax.jit
def pallas_parallel_sum__sliding_local_dilated__mixer_token_mlp__prompt_kernel(
    A_x: jax.Array,
    A_wqkv: jax.Array,
    A_wo: jax.Array,
    B_x: jax.Array,
    B_w1: jax.Array,
    B_b1: jax.Array,
    B_w2: jax.Array,
    B_b2: jax.Array,
):
    del B_x
    x = A_x.reshape(S, D).T
    any_spec = pl.BlockSpec(memory_space=pltpu.HBM)
    out = pl.pallas_call(
        _kernel,
        out_shape=jax.ShapeDtypeStruct((D, S), bf16),
        in_specs=[any_spec] * 7,
        out_specs=any_spec,
        scratch_shapes=[
            pltpu.VMEM((F,), bf16),
            pltpu.VMEM((S,), bf16),
            pltpu.VMEM((D, S), bf16),
            pltpu.VMEM((D, 3 * D), bf16),
            pltpu.VMEM((D, D), bf16),
            pltpu.VMEM((S, F), bf16),
            pltpu.VMEM((NT, F, TB), bf16),
            pltpu.VMEM((D // 2, S), u32),
            pltpu.VMEM((3 * D // 2, D), u32),
            pltpu.VMEM((D // 2, D), u32),
            pltpu.VMEM((D, F), f32),
            pltpu.VMEM((D // 2, F), u32),
            pltpu.VMEM((D // 2, S + PAD), u32),
            pltpu.VMEM((D // 2, S + PAD), u32),
            pltpu.VMEM((4, 3 * D, 128), f32),
            pltpu.VMEM((4, D, 128), f32),
            pltpu.VMEM((NT, D, TB), bf16),
            pltpu.SemaphoreType.DMA((3 * NT + 5,)),
            pltpu.SemaphoreType.DMA((NT + 7,)),
        ],
        compiler_params=pltpu.CompilerParams(vmem_limit_bytes=100 * 1024 * 1024, disable_bounds_checks=True,
                                             disable_semaphore_checks=True),
        name="fused_attn_mixer",
    )(x, A_wqkv, A_wo, B_w1, B_b1, B_w2, B_b2)
    return out.T.reshape(1, S, D)
```

```python
import contextlib
import functools

import jax
import jax.numpy as jnp
import jax.experimental.pallas as pl
import jax.experimental.pallas.tpu as pltpu

S, D, F = 2048, 448, 1792
H, DH, W, DIL = 16, 28, 8, 2
TB = 256
NT = S // TB
PAD = 128
F0 = 768

bf16 = jnp.bfloat16
f32 = jnp.float32
u32 = jnp.uint32

SCOPES = False
SWEEP = [(1,), (2,), (3,), (4, 5), (6, 7)]
ORDER = ["x0", "b1", "w1_0a", "w1_0b", "x1", "w1_1", "x2", "w1_2", "x3", "w1_3", "x4", "w1_4", "x5", "w1_5", "x6", "x7", "w1_6", "w1_7",
         "wqkv", "wo", "b2"] + ["w2_%d" % i for i in range(NT)]
SEM = {"x%d" % i: i for i in range(NT)}
SEM.update({"w1_%d" % i: NT + i for i in range(1, NT)})
SEM.update({"w2_%d" % i: 2 * NT + i for i in range(NT)})
SEM.update({"w1_0a": NT, "w1_0b": 3 * NT, "wqkv": 3 * NT + 1, "wo": 3 * NT + 2, "b1": 3 * NT + 3, "b2": 3 * NT + 4})


def _gelu(x):
    c = 0.7978845608028654
    return 0.5 * x * (1.0 + jnp.tanh(c * (x + 0.044715 * (x * x * x))))


def _pack(v):
    return pltpu.bitcast(v, u32)


def _unpack(v):
    return pltpu.bitcast(v, bf16)


def _scope(name):
    return jax.named_scope(name) if SCOPES else contextlib.nullcontext()


def _kernel(x_hbm, wqkv_hbm, wo_hbm, w1_hbm, b1_hbm, w2_hbm, b2_hbm, out_hbm,
            b1_v, b2_v, x_v, wqkv_v, wo_v, w1_v, w2_v, xnT, wqkvT, woT, acc_v, u_v, kT, vT, tmp, tmp2, out_v,
            isem, osem):
    x_hbm, wqkv_hbm, wo_hbm, w1_hbm, w2_hbm = (
        r.bitcast(u32) for r in (x_hbm, wqkv_hbm, wo_hbm, w1_hbm, w2_hbm))
    HB = TB // 2
    copies = {}
    for i in range(NT):
        copies["x%d" % i] = (x_hbm.at[:, pl.ds(i * TB, TB)], x_v.at[:, pl.ds(i * TB, TB)])
        if i > 0:
            copies["w1_%d" % i] = (w1_hbm.at[pl.ds(i * HB, HB), :], w1_v.at[pl.ds(i * HB, HB), :])
        copies["w2_%d" % i] = (w2_hbm.at[:, pl.ds(i * TB, TB)], w2_v.at[i])
    copies["w1_0a"] = (w1_hbm.at[pl.ds(0, HB), pl.ds(0, F0)], w1_v.at[pl.ds(0, HB), pl.ds(0, F0)])
    copies["w1_0b"] = (w1_hbm.at[pl.ds(0, HB), pl.ds(F0, F - F0)], w1_v.at[pl.ds(0, HB), pl.ds(F0, F - F0)])
    copies["wqkv"] = (wqkv_hbm, wqkv_v)
    copies["wo"] = (wo_hbm, wo_v)
    copies["b1"] = (b1_hbm, b1_v)
    copies["b2"] = (b2_hbm, b2_v)
    assert sorted(copies) == sorted(ORDER)
    dma = {n: pltpu.make_async_copy(copies[n][0], copies[n][1], isem.at[SEM[n]]) for n in ORDER}
    waited = set()

    def wait(*names):
        for n in names:
            if n not in waited:
                waited.add(n)
                dma[n].wait()

    def ds(i, n=1, off=0):
        if isinstance(i, int):
            return slice(i * TB + off, (i + n) * TB + off)
        return pl.ds(pl.multiple_of(i * TB + off, 128), n * TB)

    def wrows(i, n=1):
        if isinstance(i, int):
            return slice(i * HB, (i + n) * HB)
        return pl.ds(pl.multiple_of(i * HB, HB), n * HB)

    def w2_dma(j):
        return pltpu.make_async_copy(w2_hbm.at[:, ds(j)], w2_v.at[j], isem.at[W2SEM + j])

    def out_copy(j):
        return pltpu.make_async_copy(out_v.at[j], out_hbm.at[:, ds(j)], osem.at[j])

    RL = D // 7
    last_copies = [pltpu.make_async_copy(out_v.at[NT - 1, pl.ds(p * RL, RL), :],
                                         out_hbm.at[pl.ds(p * RL, RL), pl.ds((NT - 1) * TB, TB)], osem.at[NT + p]) for p in range(7)]

    def ln(i):
        xt = _unpack(x_v[:, ds(i)]).astype(f32)
        m = jnp.mean(xt, axis=0, keepdims=True)
        xc = xt - m
        v = jnp.mean(xc * xc, axis=0, keepdims=True)
        xnT[:, ds(i)] = _pack((xc * jax.lax.rsqrt(v + 1e-5)).astype(bf16))

    def prep_wqkv():
        wt = _unpack(wqkv_v[...]).astype(f32).T
        for c in range(4):
            lo, hi = 128 * c, min(128 * (c + 1), D)
            tmp[c, :, 0:hi - lo] = wt[:, lo:hi]
        for t in range(3):
            for d in range(DH):
                rows = [tmp[c, pl.ds(t * D + d, H, stride=DH), :] for c in range(4)]
                blk = jnp.concatenate(rows, axis=1)[:, :D]
                wqkvT[pl.ds((t * D + d * H) // 2, H // 2), :] = _pack(blk.astype(bf16))

    def prep_wo():
        wof = _unpack(wo_v[...]).astype(f32)
        for c in range(4):
            lo, hi = 128 * c, min(128 * (c + 1), D)
            tmp2[c, :, 0:hi - lo] = wof[:, lo:hi]
        blks = []
        for d in range(DH):
            rows = [tmp2[c, pl.ds(d, H, stride=DH), :] for c in range(4)]
            blks.append(jnp.concatenate(rows, axis=1)[:, :D])
        woT[...] = _pack(jnp.concatenate(blks, axis=0).T.astype(bf16))
        kT[:, 0:PAD] = jnp.zeros((D // 2, PAD), u32)
        vT[:, 0:PAD] = jnp.zeros((D // 2, PAD), u32)

    def sweep_first(c0, c1):
        part = jnp.dot(_unpack(xnT[:, 0:TB]), _unpack(w1_v[0:HB, c0:c1]), preferred_element_type=f32)
        acc_v[:, c0:c1] = part + b1_v[c0:c1].astype(f32)[None, :]

    def sweep(blocks, last):
        k0, k1 = blocks[0] * TB, (blocks[-1] + 1) * TB
        part = jnp.dot(_unpack(xnT[:, k0:k1]), _unpack(w1_v[k0 // 2:k1 // 2, :]), preferred_element_type=f32)
        if not last:
            acc_v[...] = acc_v[...] + part
        else:
            u_v[...] = _pack(_gelu(acc_v[...] + part).astype(bf16))

    scale = DH ** -0.5

    def qkv_mm(j):
        qkv = jnp.dot(_unpack(wqkvT[...]), _unpack(xnT[:, ds(j)]), preferred_element_type=f32)
        kT[:, ds(j, 1, PAD)] = _pack(qkv[D:2 * D].astype(bf16))
        vT[:, ds(j, 1, PAD)] = _pack(qkv[2 * D:3 * D].astype(bf16))
        return qkv[0:D]

    def y_mm(j):
        y = jnp.dot(_unpack(u_v[...]), _unpack(w2_v[j]), preferred_element_type=f32)
        return y + b2_v[ds(j)].astype(f32)[None, :]

    def window(j):
        if isinstance(j, int):
            return slice(j * TB, (j + 1) * TB + PAD)
        return pl.ds(pl.multiple_of(j * TB, 128), TB + PAD)

    def attn(j, q, first):
        kw = kT[:, window(j)]
        vw = vT[:, window(j)]
        pos = jax.lax.broadcasted_iota(jnp.int32, (H, TB), 1)
        logits = []
        for w in range(W):
            ks = kw if w == 0 else pltpu.roll(kw, DIL * w, 1)
            ks = _unpack(ks[:, PAD:]).astype(f32)
            lg = (q * ks).reshape(DH, H, TB).sum(axis=0) * scale
            logits.append(jnp.where(pos >= DIL * w, lg, -1e9) if first else lg)
        mx = functools.reduce(jnp.maximum, logits)
        es = [jnp.exp(l - mx) for l in logits]
        den = functools.reduce(jnp.add, es)
        inv = 1.0 / den
        o = None
        for w in range(W):
            vs = vw if w == 0 else pltpu.roll(vw, DIL * w, 1)
            vs = _unpack(vs[:, PAD:]).astype(f32).reshape(DH, H, TB)
            term = vs * (es[w] * inv)[None]
            o = term if o is None else o + term
        return o.reshape(D, TB).astype(bf16)

    def finish_last(j, y, oT):
        attnT = jnp.dot(_unpack(woT[...]), oT, preferred_element_type=f32)
        res = y + attnT + _unpack(x_v[:, ds(j)]).astype(f32)
        R = D // 7
        for p in range(7):
            out_v[j, p * R:(p + 1) * R, :] = res[p * R:(p + 1) * R].astype(bf16)
            last_copies[p].start()

    def finish(j, y, oT):
        attnT = jnp.dot(_unpack(woT[...]), oT, preferred_element_type=f32)
        res = y + attnT + _unpack(x_v[:, ds(j)]).astype(f32)
        out_v[j] = res.astype(bf16)
        out_copy(j).start()

    for n in ORDER:
        dma[n].start()
    with _scope("p0"):
        wait("x0")
        ln(0)
    with _scope("s0a_wait"):
        wait("b1", "w1_0a")
    with _scope("s0a"):
        sweep_first(0, F0)
    with _scope("s0b_wait"):
        wait("w1_0b", "x1")
    with _scope("s0b"):
        sweep_first(F0, F)
        ln(1)
    def sweep_body(i, c):
        pltpu.make_async_copy(w1_hbm.at[wrows(i), :], w1_v.at[wrows(i), :], isem.at[NT + i]).wait()
        pltpu.make_async_copy(x_hbm.at[:, ds(i + 1)], x_v.at[:, ds(i + 1)], isem.at[i + 1]).wait()
        part = jnp.dot(_unpack(xnT[:, ds(i)]), _unpack(w1_v[wrows(i), :]), preferred_element_type=f32)
        acc_v[...] = acc_v[...] + part
        ln(i + 1)
        return c

    with _scope("sweep_loop"):
        jax.lax.fori_loop(1, 6, sweep_body, 0)
    for i in range(1, 6):
        waited.add("w1_%d" % i)
        waited.add("x%d" % (i + 1))
    with _scope("s5_wait"):
        wait("x7", "w1_6", "w1_7", "wqkv", "wo")
    with _scope("s5"):
        p6 = jnp.dot(_unpack(xnT[:, ds(6)]), _unpack(w1_v[wrows(6), :]), preferred_element_type=f32)
        ln(7)
        p7 = jnp.dot(_unpack(xnT[:, ds(7)]), _unpack(w1_v[wrows(7), :]), preferred_element_type=f32)
        u_v[...] = _pack(_gelu(acc_v[...] + p6 + p7).astype(bf16))
        prep_wqkv()
        prep_wo()
        q = qkv_mm(0)
    with _scope("b_wait0"):
        wait("b2", "w2_0", "w2_1", "w2_2", "w2_3")
    with _scope("b0"):
        for j in range(4):
            y = y_mm(j)
            oT = attn(j, q, j == 0)
            q = qkv_mm(j + 1)
            finish(j, y, oT)
    with _scope("b_wait1"):
        wait("w2_4", "w2_5", "w2_6", "w2_7")
    with _scope("b1"):
        for j in range(4, NT):
            y = y_mm(j)
            oT = attn(j, q, False)
            if j + 1 < NT:
                q = qkv_mm(j + 1)
            (finish if j + 1 < NT else finish_last)(j, y, oT)
    with _scope("end_wait"):
        for i in range(NT - 1):
            out_copy(i).wait()
        for c in last_copies:
            c.wait()
    assert waited == set(ORDER), set(ORDER) - waited


@jax.jit
def pallas_parallel_sum__sliding_local_dilated__mixer_token_mlp__prompt_kernel(
    A_x: jax.Array,
    A_wqkv: jax.Array,
    A_wo: jax.Array,
    B_x: jax.Array,
    B_w1: jax.Array,
    B_b1: jax.Array,
    B_w2: jax.Array,
    B_b2: jax.Array,
):
    del B_x
    x = A_x.reshape(S, D).T
    any_spec = pl.BlockSpec(memory_space=pltpu.HBM)
    out = pl.pallas_call(
        _kernel,
        out_shape=jax.ShapeDtypeStruct((D, S), bf16),
        in_specs=[any_spec] * 7,
        out_specs=any_spec,
        scratch_shapes=[
            pltpu.VMEM((F,), bf16),
            pltpu.VMEM((S,), bf16),
            pltpu.VMEM((D // 2, S), u32),
            pltpu.VMEM((D // 2, 3 * D), u32),
            pltpu.VMEM((D // 2, D), u32),
            pltpu.VMEM((S // 2, F), u32),
            pltpu.VMEM((NT, F // 2, TB), u32),
            pltpu.VMEM((D // 2, S), u32),
            pltpu.VMEM((3 * D // 2, D), u32),
            pltpu.VMEM((D // 2, D), u32),
            pltpu.VMEM((D, F), f32),
            pltpu.VMEM((D // 2, F), u32),
            pltpu.VMEM((D // 2, S + PAD), u32),
            pltpu.VMEM((D // 2, S + PAD), u32),
            pltpu.VMEM((4, 3 * D, 128), f32),
            pltpu.VMEM((4, D, 128), f32),
            pltpu.VMEM((NT, D, TB), bf16),
            pltpu.SemaphoreType.DMA((3 * NT + 5,)),
            pltpu.SemaphoreType.DMA((NT + 7,)),
        ],
        compiler_params=pltpu.CompilerParams(vmem_limit_bytes=100 * 1024 * 1024, disable_bounds_checks=True,
                                             disable_semaphore_checks=True),
        name="fused_attn_mixer",
    )(x, A_wqkv, A_wo, B_w1, B_b1, B_w2, B_b2)
    return out.T.reshape(1, S, D)
```

```python
import functools

import jax
import jax.numpy as jnp
import jax.experimental.pallas as pl
import jax.experimental.pallas.tpu as pltpu

S, D, F = 2048, 448, 1792
H, DH, W, DIL = 16, 28, 8, 2
TB = 256
NT = S // TB
HB = TB // 2
PAD = 128
F0 = 768
NLAST = 7
EPS = 1e-5

bf16 = jnp.bfloat16
f32 = jnp.float32
u32 = jnp.uint32

_ORDER = (["x0", "b1", "w1_0a", "w1_0b", "x1", "w1_1", "x2", "w1_2", "x3", "w1_3", "x4", "w1_4", "x5", "w1_5",
           "x6", "x7", "w1_6", "w1_7", "wqkv", "wo", "b2"] + ["w2_%d" % i for i in range(NT)])
_SEM = {"x%d" % i: i for i in range(NT)}
_SEM.update({"w1_%d" % i: NT + i for i in range(1, NT)})
_SEM.update({"w2_%d" % i: 2 * NT + i for i in range(NT)})
_SEM.update({"w1_0a": NT, "w1_0b": 3 * NT, "wqkv": 3 * NT + 1, "wo": 3 * NT + 2, "b1": 3 * NT + 3, "b2": 3 * NT + 4})


def _gelu(x):
    c = 0.7978845608028654
    return 0.5 * x * (1.0 + jnp.tanh(c * (x + 0.044715 * (x * x * x))))


def _pack(v):
    return pltpu.bitcast(v, u32)


def _unpack(v):
    return pltpu.bitcast(v, bf16)


def _cols(i, off=0):
    if isinstance(i, int):
        return slice(i * TB + off, (i + 1) * TB + off)
    return pl.ds(pl.multiple_of(i * TB + off, 128), TB)


def _w1_rows(i):
    if isinstance(i, int):
        return slice(i * HB, (i + 1) * HB)
    return pl.ds(pl.multiple_of(i * HB, HB), HB)


def _kernel(x_hbm, wqkv_hbm, wo_hbm, w1_hbm, b1_hbm, w2_hbm, b2_hbm, out_hbm,
            b1_v, b2_v, x_v, wqkv_v, wo_v, w1_v, w2_v, xnT, wqkvT, woT, acc_v, u_v, kT, vT, tmp_qkv, tmp_o, out_v,
            isem, osem):
    x_hbm, wqkv_hbm, wo_hbm, w1_hbm, w2_hbm = (
        r.bitcast(u32) for r in (x_hbm, wqkv_hbm, wo_hbm, w1_hbm, w2_hbm))

    copies = {
        "w1_0a": (w1_hbm.at[pl.ds(0, HB), pl.ds(0, F0)], w1_v.at[pl.ds(0, HB), pl.ds(0, F0)]),
        "w1_0b": (w1_hbm.at[pl.ds(0, HB), pl.ds(F0, F - F0)], w1_v.at[pl.ds(0, HB), pl.ds(F0, F - F0)]),
        "wqkv": (wqkv_hbm, wqkv_v), "wo": (wo_hbm, wo_v), "b1": (b1_hbm, b1_v), "b2": (b2_hbm, b2_v),
    }
    for i in range(NT):
        copies["x%d" % i] = (x_hbm.at[:, pl.ds(i * TB, TB)], x_v.at[:, pl.ds(i * TB, TB)])
        copies["w2_%d" % i] = (w2_hbm.at[:, pl.ds(i * TB, TB)], w2_v.at[i])
        if i > 0:
            copies["w1_%d" % i] = (w1_hbm.at[pl.ds(i * HB, HB), :], w1_v.at[pl.ds(i * HB, HB), :])
    dma = {n: pltpu.make_async_copy(copies[n][0], copies[n][1], isem.at[_SEM[n]]) for n in _ORDER}

    def wait(*names):
        for n in names:
            dma[n].wait()

    def out_copy(j):
        return pltpu.make_async_copy(out_v.at[j], out_hbm.at[:, _cols(j)], osem.at[j])

    RL = D // NLAST
    last_copies = [
        pltpu.make_async_copy(out_v.at[NT - 1, pl.ds(p * RL, RL), :],
                              out_hbm.at[pl.ds(p * RL, RL), pl.ds((NT - 1) * TB, TB)], osem.at[NT - 1 + p])
        for p in range(NLAST)]

    def layer_norm(i):
        xt = _unpack(x_v[:, _cols(i)]).astype(f32)
        m = jnp.mean(xt, axis=0, keepdims=True)
        xc = xt - m
        v = jnp.mean(xc * xc, axis=0, keepdims=True)
        xnT[:, _cols(i)] = _pack((xc * jax.lax.rsqrt(v + EPS)).astype(bf16))

    def mix1(i, c0=0, c1=F):
        return jnp.dot(_unpack(xnT[:, _cols(i)]), _unpack(w1_v[_w1_rows(i), c0:c1]), preferred_element_type=f32)

    def prep_wqkv():
        wt = _unpack(wqkv_v[...]).astype(f32).T
        for c in range(4):
            lo, hi = 128 * c, min(128 * (c + 1), D)
            tmp_qkv[c, :, 0:hi - lo] = wt[:, lo:hi]
        for t in range(3):
            for d in range(DH):
                rows = [tmp_qkv[c, pl.ds(t * D + d, H, stride=DH), :] for c in range(4)]
                blk = jnp.concatenate(rows, axis=1)[:, :D]
                wqkvT[pl.ds((t * D + d * H) // 2, H // 2), :] = _pack(blk.astype(bf16))

    def prep_wo():
        wof = _unpack(wo_v[...]).astype(f32)
        for c in range(4):
            lo, hi = 128 * c, min(128 * (c + 1), D)
            tmp_o[c, :, 0:hi - lo] = wof[:, lo:hi]
        blks = []
        for d in range(DH):
            rows = [tmp_o[c, pl.ds(d, H, stride=DH), :] for c in range(4)]
            blks.append(jnp.concatenate(rows, axis=1)[:, :D])
        woT[...] = _pack(jnp.concatenate(blks, axis=0).T.astype(bf16))
        kT[:, 0:PAD] = jnp.zeros((D // 2, PAD), u32)
        vT[:, 0:PAD] = jnp.zeros((D // 2, PAD), u32)

    def qkv_proj(j):
        qkv = jnp.dot(_unpack(wqkvT[...]), _unpack(xnT[:, _cols(j)]), preferred_element_type=f32)
        kT[:, _cols(j, PAD)] = _pack(qkv[D:2 * D].astype(bf16))
        vT[:, _cols(j, PAD)] = _pack(qkv[2 * D:3 * D].astype(bf16))
        return qkv[0:D]

    def mix2(j):
        y = jnp.dot(_unpack(u_v[...]), _unpack(w2_v[j]), preferred_element_type=f32)
        return y + b2_v[_cols(j)].astype(f32)[None, :]

    def attention(j, q):
        win = slice(j * TB, (j + 1) * TB + PAD)
        kw = kT[:, win]
        vw = vT[:, win]
        pos = j * TB + jax.lax.broadcasted_iota(jnp.int32, (H, TB), 1)
        scale = DH ** -0.5
        logits = []
        for w in range(W):
            ks = kw if w == 0 else pltpu.roll(kw, DIL * w, 1)
            ks = _unpack(ks[:, PAD:]).astype(f32)
            lg = (q * ks).reshape(DH, H, TB).sum(axis=0) * scale
            if j * TB < DIL * w:
                lg = jnp.where(pos >= DIL * w, lg, -1e9)
            logits.append(lg)
        mx = functools.reduce(jnp.maximum, logits)
        es = [jnp.exp(l - mx) for l in logits]
        inv = 1.0 / functools.reduce(jnp.add, es)
        o = None
        for w in range(W):
            vs = vw if w == 0 else pltpu.roll(vw, DIL * w, 1)
            vs = _unpack(vs[:, PAD:]).astype(f32).reshape(DH, H, TB)
            term = vs * (es[w] * inv)[None]
            o = term if o is None else o + term
        return o.reshape(D, TB).astype(bf16)

    def finish(j, y, oT):
        attnT = jnp.dot(_unpack(woT[...]), oT, preferred_element_type=f32)
        res = y + attnT + _unpack(x_v[:, _cols(j)]).astype(f32)
        if j < NT - 1:
            out_v[j] = res.astype(bf16)
            out_copy(j).start()
        else:
            for p in range(NLAST):
                out_v[j, p * RL:(p + 1) * RL, :] = res[p * RL:(p + 1) * RL].astype(bf16)
                last_copies[p].start()

    for n in _ORDER:
        dma[n].start()
    wait("x0")
    layer_norm(0)
    wait("b1", "w1_0a")
    acc_v[:, 0:F0] = mix1(0, 0, F0) + b1_v[0:F0].astype(f32)[None, :]
    wait("w1_0b", "x1")
    acc_v[:, F0:F] = mix1(0, F0, F) + b1_v[F0:F].astype(f32)[None, :]
    layer_norm(1)

    def sweep(i, carry):
        pltpu.make_async_copy(w1_hbm.at[_w1_rows(i), :], w1_v.at[_w1_rows(i), :], isem.at[NT + i]).wait()
        pltpu.make_async_copy(x_hbm.at[:, _cols(i + 1)], x_v.at[:, _cols(i + 1)], isem.at[i + 1]).wait()
        acc_v[...] = acc_v[...] + mix1(i)
        layer_norm(i + 1)
        return carry

    jax.lax.fori_loop(1, NT - 2, sweep, 0)

    wait("x7", "w1_6", "w1_7", "wqkv", "wo")
    p6 = mix1(NT - 2)
    layer_norm(NT - 1)
    p7 = mix1(NT - 1)
    u_v[...] = _pack(_gelu(acc_v[...] + p6 + p7).astype(bf16))
    prep_wqkv()
    prep_wo()
    q = qkv_proj(0)

    for j in range(NT):
        if j == 0:
            wait("b2", "w2_0", "w2_1", "w2_2", "w2_3")
        if j == NT // 2:
            wait("w2_4", "w2_5", "w2_6", "w2_7")
        y = mix2(j)
        oT = attention(j, q)
        if j + 1 < NT:
            q = qkv_proj(j + 1)
        finish(j, y, oT)

    for j in range(NT - 1):
        out_copy(j).wait()
    for c in last_copies:
        c.wait()


@jax.jit
def pallas_parallel_sum__sliding_local_dilated__mixer_token_mlp__prompt_kernel(
    A_x: jax.Array,
    A_wqkv: jax.Array,
    A_wo: jax.Array,
    B_x: jax.Array,
    B_w1: jax.Array,
    B_b1: jax.Array,
    B_w2: jax.Array,
    B_b2: jax.Array,
):
    del B_x
    xT = A_x.reshape(S, D).T
    hbm = pl.BlockSpec(memory_space=pltpu.HBM)
    outT = pl.pallas_call(
        _kernel,
        out_shape=jax.ShapeDtypeStruct((D, S), bf16),
        in_specs=[hbm] * 7,
        out_specs=hbm,
        scratch_shapes=[
            pltpu.VMEM((F,), bf16),
            pltpu.VMEM((S,), bf16),
            pltpu.VMEM((D // 2, S), u32),
            pltpu.VMEM((D // 2, 3 * D), u32),
            pltpu.VMEM((D // 2, D), u32),
            pltpu.VMEM((S // 2, F), u32),
            pltpu.VMEM((NT, F // 2, TB), u32),
            pltpu.VMEM((D // 2, S), u32),
            pltpu.VMEM((3 * D // 2, D), u32),
            pltpu.VMEM((D // 2, D), u32),
            pltpu.VMEM((D, F), f32),
            pltpu.VMEM((D // 2, F), u32),
            pltpu.VMEM((D // 2, S + PAD), u32),
            pltpu.VMEM((D // 2, S + PAD), u32),
            pltpu.VMEM((4, 3 * D, 128), f32),
            pltpu.VMEM((4, D, 128), f32),
            pltpu.VMEM((NT, D, TB), bf16),
            pltpu.SemaphoreType.DMA((3 * NT + 5,)),
            pltpu.SemaphoreType.DMA((NT - 1 + NLAST,)),
        ],
        compiler_params=pltpu.CompilerParams(
            vmem_limit_bytes=100 * 1024 * 1024, disable_bounds_checks=True, disable_semaphore_checks=True),
        name="fused_attn_mixer",
    )(xT, A_wqkv, A_wo, B_w1, B_b1, B_w2, B_b2)
    return outT.T.reshape(1, S, D)
```

```python
import functools

import jax
import jax.numpy as jnp
import jax.experimental.pallas as pl
import jax.experimental.pallas.tpu as pltpu

S, D, F = 2048, 448, 1792
H, DH, W, DIL = 16, 28, 8, 2
TB = 256
NT = S // TB
HB = TB // 2
PAD = 128
F0 = 768
NLAST = 7
EPS = 1e-5

bf16 = jnp.bfloat16
f32 = jnp.float32
u32 = jnp.uint32

_ORDER = (["x0", "b1", "w1_0a", "w1_0b", "x1", "w1_1", "x2", "w1_2", "x3", "w1_3", "x4", "w1_4", "x5", "w1_5",
           "x6", "x7", "w1_6", "w1_7", "wqkv", "wo", "b2"] + ["w2_%d" % i for i in range(NT)])
_SEM = {"x%d" % i: i for i in range(NT)}
_SEM.update({"w1_%d" % i: NT + i for i in range(1, NT)})
_SEM.update({"w2_%d" % i: 2 * NT + i for i in range(NT)})
_SEM.update({"w1_0a": NT, "w1_0b": 3 * NT, "wqkv": 3 * NT + 1, "wo": 3 * NT + 2, "b1": 3 * NT + 3, "b2": 3 * NT + 4})


def _gelu(x):
    c = 0.7978845608028654
    return 0.5 * x * (1.0 + jnp.tanh(c * (x + 0.044715 * (x * x * x))))


def _pack(v):
    return pltpu.bitcast(v, u32)


def _unpack(v):
    return pltpu.bitcast(v, bf16)


def _cols(i, off=0):
    if isinstance(i, int):
        return slice(i * TB + off, (i + 1) * TB + off)
    return pl.ds(pl.multiple_of(i * TB + off, 128), TB)


def _w1_rows(i):
    if isinstance(i, int):
        return slice(i * HB, (i + 1) * HB)
    return pl.ds(pl.multiple_of(i * HB, HB), HB)


def _kernel(x_hbm, wqkv_hbm, wo_hbm, w1_hbm, b1_hbm, w2_hbm, b2_hbm, out_hbm,
            b1_v, b2_v, x_v, wqkv_v, wo_v, w1_v, w2_v, xnT, wqkvT, woT, acc_v, u_v, kT, vT, tmp_qkv, tmp_o, out_v,
            isem, osem):
    x_hbm, wqkv_hbm, wo_hbm, w1_hbm, w2_hbm = (
        r.bitcast(u32) for r in (x_hbm, wqkv_hbm, wo_hbm, w1_hbm, w2_hbm))

    copies = {
        "w1_0a": (w1_hbm.at[pl.ds(0, HB), pl.ds(0, F0)], w1_v.at[pl.ds(0, HB), pl.ds(0, F0)]),
        "w1_0b": (w1_hbm.at[pl.ds(0, HB), pl.ds(F0, F - F0)], w1_v.at[pl.ds(0, HB), pl.ds(F0, F - F0)]),
        "wqkv": (wqkv_hbm, wqkv_v), "wo": (wo_hbm, wo_v), "b1": (b1_hbm, b1_v), "b2": (b2_hbm, b2_v),
    }
    for i in range(NT):
        copies["x%d" % i] = (x_hbm.at[:, pl.ds(i * TB, TB)], x_v.at[:, pl.ds(i * TB, TB)])
        copies["w2_%d" % i] = (w2_hbm.at[:, pl.ds(i * TB, TB)], w2_v.at[i])
        if i > 0:
            copies["w1_%d" % i] = (w1_hbm.at[pl.ds(i * HB, HB), :], w1_v.at[pl.ds(i * HB, HB), :])
    dma = {n: pltpu.make_async_copy(copies[n][0], copies[n][1], isem.at[_SEM[n]]) for n in _ORDER}

    def wait(*names):
        for n in names:
            dma[n].wait()

    def out_copy(j):
        return pltpu.make_async_copy(out_v.at[j], out_hbm.at[:, _cols(j)], osem.at[j])

    RL = D // NLAST
    last_copies = [
        pltpu.make_async_copy(out_v.at[NT - 1, pl.ds(p * RL, RL), :],
                              out_hbm.at[pl.ds(p * RL, RL), pl.ds((NT - 1) * TB, TB)], osem.at[NT - 1 + p])
        for p in range(NLAST)]

    def layer_norm(i):
        xt = _unpack(x_v[:, _cols(i)]).astype(f32)
        m = jnp.mean(xt, axis=0, keepdims=True)
        xc = xt - m
        v = jnp.mean(xc * xc, axis=0, keepdims=True)
        xnT[:, _cols(i)] = _pack((xc * jax.lax.rsqrt(v + EPS)).astype(bf16))

    def mix1(i, c0=0, c1=F):
        return jnp.dot(_unpack(xnT[:, _cols(i)]), _unpack(w1_v[_w1_rows(i), c0:c1]), preferred_element_type=f32)

    def prep_wqkv():
        wt = _unpack(wqkv_v[...]).astype(f32).T
        for c in range(4):
            lo, hi = 128 * c, min(128 * (c + 1), D)
            tmp_qkv[c, :, 0:hi - lo] = wt[:, lo:hi]
        for t in range(3):
            for d in range(DH):
                rows = [tmp_qkv[c, pl.ds(t * D + d, H, stride=DH), 0:min(128, D - 128 * c)] for c in range(4)]
                blk = jnp.concatenate(rows, axis=1)
                wqkvT[pl.ds((t * D + d * H) // 2, H // 2), :] = _pack(blk.astype(bf16))

    def prep_wo():
        wof = _unpack(wo_v[...]).astype(f32)
        for c in range(4):
            lo, hi = 128 * c, min(128 * (c + 1), D)
            tmp_o[c, :, 0:hi - lo] = wof[:, lo:hi]
        blks = []
        for d in range(DH):
            rows = [tmp_o[c, pl.ds(d, H, stride=DH), 0:min(128, D - 128 * c)] for c in range(4)]
            blks.append(jnp.concatenate(rows, axis=1))
        woT[...] = _pack(jnp.concatenate(blks, axis=0).T.astype(bf16))
        kT[:, 0:PAD] = jnp.zeros((D // 2, PAD), u32)
        vT[:, 0:PAD] = jnp.zeros((D // 2, PAD), u32)

    def qkv_proj(j):
        qkv = jnp.dot(_unpack(wqkvT[...]), _unpack(xnT[:, _cols(j)]), preferred_element_type=f32)
        kT[:, _cols(j, PAD)] = _pack(qkv[D:2 * D].astype(bf16))
        vT[:, _cols(j, PAD)] = _pack(qkv[2 * D:3 * D].astype(bf16))
        return qkv[0:D]

    def mix2(j):
        y = jnp.dot(_unpack(u_v[...]), _unpack(w2_v[j]), preferred_element_type=f32)
        return y + b2_v[_cols(j)].astype(f32)[None, :]

    def attention(j, q):
        win = slice(j * TB, (j + 1) * TB + PAD)
        kw = kT[:, win]
        vw = vT[:, win]
        pos = j * TB + jax.lax.broadcasted_iota(jnp.int32, (H, TB), 1)
        scale = DH ** -0.5
        logits = []
        for w in range(W):
            ks = kw if w == 0 else pltpu.roll(kw, DIL * w, 1)
            ks = _unpack(ks[:, PAD:]).astype(f32)
            lg = (q * ks).reshape(DH, H, TB).sum(axis=0) * scale
            if j * TB < DIL * w:
                lg = jnp.where(pos >= DIL * w, lg, -1e9)
            logits.append(lg)
        mx = functools.reduce(jnp.maximum, logits)
        es = [jnp.exp(l - mx) for l in logits]
        inv = 1.0 / functools.reduce(jnp.add, es)
        o = None
        for w in range(W):
            vs = vw if w == 0 else pltpu.roll(vw, DIL * w, 1)
            vs = _unpack(vs[:, PAD:]).astype(f32).reshape(DH, H, TB)
            term = vs * (es[w] * inv)[None]
            o = term if o is None else o + term
        return o.reshape(D, TB).astype(bf16)

    def finish(j, y, oT):
        attnT = jnp.dot(_unpack(woT[...]), oT, preferred_element_type=f32)
        res = y + attnT + _unpack(x_v[:, _cols(j)]).astype(f32)
        if j < NT - 1:
            out_v[j] = res.astype(bf16)
            out_copy(j).start()
        else:
            for p in range(NLAST):
                out_v[j, p * RL:(p + 1) * RL, :] = res[p * RL:(p + 1) * RL].astype(bf16)
                last_copies[p].start()

    for n in _ORDER:
        dma[n].start()
    wait("x0")
    layer_norm(0)
    wait("b1", "w1_0a")
    acc_v[:, 0:F0] = mix1(0, 0, F0) + b1_v[0:F0].astype(f32)[None, :]
    wait("w1_0b", "x1")
    acc_v[:, F0:F] = mix1(0, F0, F) + b1_v[F0:F].astype(f32)[None, :]
    layer_norm(1)

    def sweep(i, carry):
        pltpu.make_async_copy(w1_hbm.at[_w1_rows(i), :], w1_v.at[_w1_rows(i), :], isem.at[NT + i]).wait()
        pltpu.make_async_copy(x_hbm.at[:, _cols(i + 1)], x_v.at[:, _cols(i + 1)], isem.at[i + 1]).wait()
        acc_v[...] = acc_v[...] + mix1(i)
        layer_norm(i + 1)
        return carry

    jax.lax.fori_loop(1, NT - 2, sweep, 0)

    wait("x7", "w1_6", "w1_7", "wqkv", "wo")
    p6 = mix1(NT - 2)
    layer_norm(NT - 1)
    p7 = mix1(NT - 1)
    u_v[...] = _pack(_gelu(acc_v[...] + p6 + p7).astype(bf16))
    prep_wqkv()
    prep_wo()
    q = qkv_proj(0)

    for j in range(NT):
        if j == 0:
            wait("b2", "w2_0", "w2_1", "w2_2", "w2_3")
        if j == NT // 2:
            wait("w2_4", "w2_5", "w2_6", "w2_7")
        y = mix2(j)
        oT = attention(j, q)
        if j + 1 < NT:
            q = qkv_proj(j + 1)
        finish(j, y, oT)

    for j in range(NT - 1):
        out_copy(j).wait()
    for c in last_copies:
        c.wait()


@jax.jit
def pallas_parallel_sum__sliding_local_dilated__mixer_token_mlp__prompt_kernel(
    A_x: jax.Array,
    A_wqkv: jax.Array,
    A_wo: jax.Array,
    B_x: jax.Array,
    B_w1: jax.Array,
    B_b1: jax.Array,
    B_w2: jax.Array,
    B_b2: jax.Array,
):
    del B_x
    xT = A_x.reshape(S, D).T
    hbm = pl.BlockSpec(memory_space=pltpu.HBM)
    outT = pl.pallas_call(
        _kernel,
        out_shape=jax.ShapeDtypeStruct((D, S), bf16),
        in_specs=[hbm] * 7,
        out_specs=hbm,
        scratch_shapes=[
            pltpu.VMEM((F,), bf16),
            pltpu.VMEM((S,), bf16),
            pltpu.VMEM((D // 2, S), u32),
            pltpu.VMEM((D // 2, 3 * D), u32),
            pltpu.VMEM((D // 2, D), u32),
            pltpu.VMEM((S // 2, F), u32),
            pltpu.VMEM((NT, F // 2, TB), u32),
            pltpu.VMEM((D // 2, S), u32),
            pltpu.VMEM((3 * D // 2, D), u32),
            pltpu.VMEM((D // 2, D), u32),
            pltpu.VMEM((D, F), f32),
            pltpu.VMEM((D // 2, F), u32),
            pltpu.VMEM((D // 2, S + PAD), u32),
            pltpu.VMEM((D // 2, S + PAD), u32),
            pltpu.VMEM((4, 3 * D, 128), f32),
            pltpu.VMEM((4, D, 128), f32),
            pltpu.VMEM((NT, D, TB), bf16),
            pltpu.SemaphoreType.DMA((3 * NT + 5,)),
            pltpu.SemaphoreType.DMA((NT - 1 + NLAST,)),
        ],
        compiler_params=pltpu.CompilerParams(
            vmem_limit_bytes=100 * 1024 * 1024, disable_bounds_checks=True, disable_semaphore_checks=True),
        name="fused_attn_mixer",
    )(xT, A_wqkv, A_wo, B_w1, B_b1, B_w2, B_b2)
    return outT.T.reshape(1, S, D)
```

```python
import functools

import jax
import jax.numpy as jnp
import jax.experimental.pallas as pl
import jax.experimental.pallas.tpu as pltpu

S, D, F = 2048, 448, 1792
H, DH, W, DIL = 16, 28, 8, 2
TB = 256
NT = S // TB
HB = TB // 2
PAD = 128
F0 = 1024
NLAST = 7
EPS = 1e-5

bf16 = jnp.bfloat16
f32 = jnp.float32
u32 = jnp.uint32

_ORDER = (["x0", "b1", "w1_0a", "w1_0b", "x1", "w1_1", "x2", "w1_2", "x3", "w1_3", "x4", "w1_4", "x5", "w1_5",
           "x6", "x7", "w1_6", "w1_7", "wqkv", "wo", "b2"] + ["w2_%d" % i for i in range(NT)])
_SEM = {"x%d" % i: i for i in range(NT)}
_SEM.update({"w1_%d" % i: NT + i for i in range(1, NT)})
_SEM.update({"w2_%d" % i: 2 * NT + i for i in range(NT)})
_SEM.update({"w1_0a": NT, "w1_0b": 3 * NT, "wqkv": 3 * NT + 1, "wo": 3 * NT + 2, "b1": 3 * NT + 3,
             "b2": 3 * NT + 4, "fence": 3 * NT + 5})


def _gelu(x):
    c = 0.7978845608028654
    return 0.5 * x * (1.0 + jnp.tanh(c * (x + 0.044715 * (x * x * x))))


def _pack(v):
    return pltpu.bitcast(v, u32)


def _unpack(v):
    return pltpu.bitcast(v, bf16)


def _cols(i, off=0):
    if isinstance(i, int):
        return slice(i * TB + off, (i + 1) * TB + off)
    return pl.ds(pl.multiple_of(i * TB + off, 128), TB)


def _w1_rows(i):
    if isinstance(i, int):
        return slice(i * HB, (i + 1) * HB)
    return pl.ds(pl.multiple_of(i * HB, HB), HB)


def _kernel(x_hbm, wqkv_hbm, wo_hbm, w1_hbm, b1_hbm, w2_hbm, b2_hbm, out_hbm,
            b1_v, b2_v, x_v, wqkv_v, wo_v, w1_v, w2_v, xnT, wqkvT, woT, acc_v, u_v, kT, vT, tmp_qkv, tmp_o, out_v, fence_v,
            isem, osem):
    x_hbm, wqkv_hbm, wo_hbm, w1_hbm, w2_hbm = (
        r.bitcast(u32) for r in (x_hbm, wqkv_hbm, wo_hbm, w1_hbm, w2_hbm))

    copies = {
        "w1_0a": (w1_hbm.at[pl.ds(0, HB), pl.ds(0, F0)], w1_v.at[pl.ds(0, HB), pl.ds(0, F0)]),
        "w1_0b": (w1_hbm.at[pl.ds(0, HB), pl.ds(F0, F - F0)], w1_v.at[pl.ds(0, HB), pl.ds(F0, F - F0)]),
        "wqkv": (wqkv_hbm, wqkv_v), "wo": (wo_hbm, wo_v), "b1": (b1_hbm, b1_v), "b2": (b2_hbm, b2_v),
    }
    for i in range(NT):
        copies["x%d" % i] = (x_hbm.at[:, pl.ds(i * TB, TB)], x_v.at[:, pl.ds(i * TB, TB)])
        copies["w2_%d" % i] = (w2_hbm.at[:, pl.ds(i * TB, TB)], w2_v.at[i])
        if i > 0:
            copies["w1_%d" % i] = (w1_hbm.at[pl.ds(i * HB, HB), :], w1_v.at[pl.ds(i * HB, HB), :])
    dma = {n: pltpu.make_async_copy(copies[n][0], copies[n][1], isem.at[_SEM[n]]) for n in _ORDER}

    def wait(*names):
        for n in names:
            dma[n].wait()

    def out_copy(j):
        return pltpu.make_async_copy(out_v.at[j], out_hbm.at[:, _cols(j)], osem.at[j])

    RL = D // NLAST
    last_copies = [
        pltpu.make_async_copy(out_v.at[NT - 1, pl.ds(p * RL, RL), :],
                              out_hbm.at[pl.ds(p * RL, RL), pl.ds((NT - 1) * TB, TB)], osem.at[NT - 1 + p])
        for p in range(NLAST)]

    def layer_norm(i):
        xt = _unpack(x_v[:, _cols(i)]).astype(f32)
        m = jnp.mean(xt, axis=0, keepdims=True)
        xc = xt - m
        v = jnp.mean(xc * xc, axis=0, keepdims=True)
        xnT[:, _cols(i)] = _pack((xc * jax.lax.rsqrt(v + EPS)).astype(bf16))

    def mix1(i, c0=0, c1=F):
        return jnp.dot(_unpack(xnT[:, _cols(i)]), _unpack(w1_v[_w1_rows(i), c0:c1]), preferred_element_type=f32)

    def prep_wqkv():
        wt = _unpack(wqkv_v[...]).astype(f32).T
        for c in range(4):
            lo, hi = 128 * c, min(128 * (c + 1), D)
            tmp_qkv[c, :, 0:hi - lo] = wt[:, lo:hi]
        for t in range(3):
            for d in range(DH):
                rows = [tmp_qkv[c, pl.ds(t * D + d, H, stride=DH), 0:min(128, D - 128 * c)] for c in range(4)]
                blk = jnp.concatenate(rows, axis=1)
                wqkvT[pl.ds((t * D + d * H) // 2, H // 2), :] = _pack(blk.astype(bf16))

    def prep_wo():
        wof = _unpack(wo_v[...]).astype(f32)
        for c in range(4):
            lo, hi = 128 * c, min(128 * (c + 1), D)
            tmp_o[c, :, 0:hi - lo] = wof[:, lo:hi]
        blks = []
        for d in range(DH):
            rows = [tmp_o[c, pl.ds(d, H, stride=DH), 0:min(128, D - 128 * c)] for c in range(4)]
            blks.append(jnp.concatenate(rows, axis=1))
        woT[...] = _pack(jnp.concatenate(blks, axis=0).T.astype(bf16))
        kT[:, 0:PAD] = jnp.zeros((D // 2, PAD), u32)
        vT[:, 0:PAD] = jnp.zeros((D // 2, PAD), u32)

    def qkv_proj(j):
        qkv = jnp.dot(_unpack(wqkvT[...]), _unpack(xnT[:, _cols(j)]), preferred_element_type=f32)
        kT[:, _cols(j, PAD)] = _pack(qkv[D:2 * D].astype(bf16))
        vT[:, _cols(j, PAD)] = _pack(qkv[2 * D:3 * D].astype(bf16))
        return qkv[0:D]

    def mix2(j):
        y = jnp.dot(_unpack(u_v[...]), _unpack(w2_v[j]), preferred_element_type=f32)
        return y + b2_v[_cols(j)].astype(f32)[None, :]

    def attention(j, q):
        win = slice(j * TB, (j + 1) * TB + PAD)
        kw = kT[:, win]
        vw = vT[:, win]
        pos = j * TB + jax.lax.broadcasted_iota(jnp.int32, (H, TB), 1)
        scale = DH ** -0.5
        logits = []
        for w in range(W):
            ks = kw if w == 0 else pltpu.roll(kw, DIL * w, 1)
            ks = _unpack(ks[:, PAD:]).astype(f32)
            lg = (q * ks).reshape(DH, H, TB).sum(axis=0) * scale
            if j * TB < DIL * w:
                lg = jnp.where(pos >= DIL * w, lg, -1e9)
            logits.append(lg)
        mx = functools.reduce(jnp.maximum, logits)
        es = [jnp.exp(l - mx) for l in logits]
        inv = 1.0 / functools.reduce(jnp.add, es)
        o = None
        for w in range(W):
            vs = vw if w == 0 else pltpu.roll(vw, DIL * w, 1)
            vs = _unpack(vs[:, PAD:]).astype(f32).reshape(DH, H, TB)
            term = vs * (es[w] * inv)[None]
            o = term if o is None else o + term
        return o.reshape(D, TB).astype(bf16)

    def finish(j, y, oT):
        attnT = jnp.dot(_unpack(woT[...]), oT, preferred_element_type=f32)
        res = y + attnT + _unpack(x_v[:, _cols(j)]).astype(f32)
        if j < NT - 1:
            out_v[j] = res.astype(bf16)
            out_copy(j).start()
        else:
            for p in range(NLAST):
                out_v[j, p * RL:(p + 1) * RL, :] = res[p * RL:(p + 1) * RL].astype(bf16)
                last_copies[p].start()

    for n in _ORDER:
        dma[n].start()
    wait("x0")
    layer_norm(0)
    fence = pltpu.make_async_copy(xnT.at[pl.ds(D // 2 - 8, 8), pl.ds(128, 128)], fence_v, isem.at[_SEM["fence"]])
    fence.start()
    wait("b1", "w1_0a")
    acc_v[:, 0:F0] = mix1(0, 0, F0) + b1_v[0:F0].astype(f32)[None, :]
    wait("w1_0b", "x1")
    fence.wait()
    acc_v[:, F0:F] = mix1(0, F0, F) + b1_v[F0:F].astype(f32)[None, :]
    layer_norm(1)

    def sweep(i, carry):
        pltpu.make_async_copy(w1_hbm.at[_w1_rows(i), :], w1_v.at[_w1_rows(i), :], isem.at[NT + i]).wait()
        pltpu.make_async_copy(x_hbm.at[:, _cols(i + 1)], x_v.at[:, _cols(i + 1)], isem.at[i + 1]).wait()
        acc_v[...] = acc_v[...] + mix1(i)
        layer_norm(i + 1)
        return carry

    jax.lax.fori_loop(1, NT - 2, sweep, 0)

    wait("x7", "w1_6", "w1_7", "wqkv", "wo")
    p6 = mix1(NT - 2)
    layer_norm(NT - 1)
    p7 = mix1(NT - 1)
    u_v[...] = _pack(_gelu(acc_v[...] + p6 + p7).astype(bf16))
    prep_wqkv()
    prep_wo()
    q = qkv_proj(0)

    for j in range(NT):
        if j == 0:
            wait("b2", "w2_0", "w2_1")
        if j == 2:
            wait("w2_2", "w2_3", "w2_4", "w2_5", "w2_6", "w2_7")
        y = mix2(j)
        oT = attention(j, q)
        if j + 1 < NT:
            q = qkv_proj(j + 1)
        finish(j, y, oT)

    for j in range(NT - 1):
        out_copy(j).wait()
    for c in last_copies:
        c.wait()


@jax.jit
def pallas_parallel_sum__sliding_local_dilated__mixer_token_mlp__prompt_kernel(
    A_x: jax.Array,
    A_wqkv: jax.Array,
    A_wo: jax.Array,
    B_x: jax.Array,
    B_w1: jax.Array,
    B_b1: jax.Array,
    B_w2: jax.Array,
    B_b2: jax.Array,
):
    del B_x
    xT = A_x.reshape(S, D).T
    hbm = pl.BlockSpec(memory_space=pltpu.HBM)
    outT = pl.pallas_call(
        _kernel,
        out_shape=jax.ShapeDtypeStruct((D, S), bf16),
        in_specs=[hbm] * 7,
        out_specs=hbm,
        scratch_shapes=[
            pltpu.VMEM((F,), bf16),
            pltpu.VMEM((S,), bf16),
            pltpu.VMEM((D // 2, S), u32),
            pltpu.VMEM((D // 2, 3 * D), u32),
            pltpu.VMEM((D // 2, D), u32),
            pltpu.VMEM((S // 2, F), u32),
            pltpu.VMEM((NT, F // 2, TB), u32),
            pltpu.VMEM((D // 2, S), u32),
            pltpu.VMEM((3 * D // 2, D), u32),
            pltpu.VMEM((D // 2, D), u32),
            pltpu.VMEM((D, F), f32),
            pltpu.VMEM((D // 2, F), u32),
            pltpu.VMEM((D // 2, S + PAD), u32),
            pltpu.VMEM((D // 2, S + PAD), u32),
            pltpu.VMEM((4, 3 * D, 128), f32),
            pltpu.VMEM((4, D, 128), f32),
            pltpu.VMEM((NT, D, TB), bf16),
            pltpu.VMEM((8, 128), u32),
            pltpu.SemaphoreType.DMA((3 * NT + 6,)),
            pltpu.SemaphoreType.DMA((NT - 1 + NLAST,)),
        ],
        compiler_params=pltpu.CompilerParams(
            vmem_limit_bytes=100 * 1024 * 1024, disable_bounds_checks=True, disable_semaphore_checks=True,
            flags={"XLA_TPU_RESCHEDULE_DMA_DONES": True}),
        name="fused_attn_mixer",
    )(xT, A_wqkv, A_wo, B_w1, B_b1, B_w2, B_b2)
    return outT.T.reshape(1, S, D)
```

```python
import functools

import jax
import jax.numpy as jnp
import jax.experimental.pallas as pl
import jax.experimental.pallas.tpu as pltpu

S, D, F = 2048, 448, 1792
H, DH, W, DIL = 16, 28, 8, 2
TB = 256
NT = S // TB
HB = TB // 2
PAD = 128
F0 = 1024
NLAST = 7
EPS = 1e-5

bf16 = jnp.bfloat16
f32 = jnp.float32
u32 = jnp.uint32

_ORDER = (["x0", "b1", "w1_0a", "w1_0b", "x1", "w1_1", "x2", "w1_2", "x3", "w1_3", "x4", "w1_4", "x5", "w1_5",
           "x6", "x7", "w1_6", "w1_7", "wqkv", "wo", "b2"] + ["w2_%d" % i for i in range(NT)])
_SEM = {"x%d" % i: i for i in range(NT)}
_SEM.update({"w1_%d" % i: NT + i for i in range(1, NT)})
_SEM.update({"w2_%d" % i: 2 * NT + i for i in range(NT)})
_SEM.update({"w1_0a": NT, "w1_0b": 3 * NT, "wqkv": 3 * NT + 1, "wo": 3 * NT + 2, "b1": 3 * NT + 3,
             "b2": 3 * NT + 4, "fence": 3 * NT + 5})


def _gelu(x):
    c = 0.7978845608028654
    return 0.5 * x * (1.0 + jnp.tanh(c * (x + 0.044715 * (x * x * x))))


def _pack(v):
    return pltpu.bitcast(v, u32)


def _unpack(v):
    return pltpu.bitcast(v, bf16)


def _cols(i, off=0):
    if isinstance(i, int):
        return slice(i * TB + off, (i + 1) * TB + off)
    return pl.ds(pl.multiple_of(i * TB + off, 128), TB)


def _w1_rows(i):
    if isinstance(i, int):
        return slice(i * HB, (i + 1) * HB)
    return pl.ds(pl.multiple_of(i * HB, HB), HB)


def _kernel(x_hbm, wqkv_hbm, wo_hbm, w1_hbm, b1_hbm, w2_hbm, b2_hbm, out_hbm,
            b1_v, b2_v, x_v, wqkv_v, wo_v, w1_v, w2_v, xnT, wqkvT, woT, acc_v, u_v, kT, vT, tmp_qkv, tmp_o, out_v, fence_v,
            isem, osem):
    x_hbm, wqkv_hbm, wo_hbm, w1_hbm, w2_hbm = (
        r.bitcast(u32) for r in (x_hbm, wqkv_hbm, wo_hbm, w1_hbm, w2_hbm))

    copies = {
        "w1_0a": (w1_hbm.at[pl.ds(0, HB), pl.ds(0, F0)], w1_v.at[pl.ds(0, HB), pl.ds(0, F0)]),
        "w1_0b": (w1_hbm.at[pl.ds(0, HB), pl.ds(F0, F - F0)], w1_v.at[pl.ds(0, HB), pl.ds(F0, F - F0)]),
        "wqkv": (wqkv_hbm, wqkv_v), "wo": (wo_hbm, wo_v), "b1": (b1_hbm, b1_v), "b2": (b2_hbm, b2_v),
    }
    for i in range(NT):
        copies["x%d" % i] = (x_hbm.at[:, pl.ds(i * TB, TB)], x_v.at[:, pl.ds(i * TB, TB)])
        copies["w2_%d" % i] = (w2_hbm.at[:, pl.ds(i * TB, TB)], w2_v.at[i])
        if i > 0:
            copies["w1_%d" % i] = (w1_hbm.at[pl.ds(i * HB, HB), :], w1_v.at[pl.ds(i * HB, HB), :])
    dma = {n: pltpu.make_async_copy(copies[n][0], copies[n][1], isem.at[_SEM[n]]) for n in _ORDER}

    def wait(*names):
        for n in names:
            dma[n].wait()

    def out_copy(j):
        return pltpu.make_async_copy(out_v.at[j], out_hbm.at[:, _cols(j)], osem.at[j])

    RL = D // NLAST
    last_copies = [
        pltpu.make_async_copy(out_v.at[NT - 1, pl.ds(p * RL, RL), :],
                              out_hbm.at[pl.ds(p * RL, RL), pl.ds((NT - 1) * TB, TB)], osem.at[NT - 1 + p])
        for p in range(NLAST)]

    def layer_norm(i):
        xt = _unpack(x_v[:, _cols(i)]).astype(f32)
        m = jnp.mean(xt, axis=0, keepdims=True)
        xc = xt - m
        v = jnp.mean(xc * xc, axis=0, keepdims=True)
        xnT[:, _cols(i)] = _pack((xc * jax.lax.rsqrt(v + EPS)).astype(bf16))

    def mix1(i, c0=0, c1=F):
        return jnp.dot(_unpack(xnT[:, _cols(i)]), _unpack(w1_v[_w1_rows(i), c0:c1]), preferred_element_type=f32)

    def prep_wqkv():
        wt = _unpack(wqkv_v[...]).astype(f32).T
        for c in range(4):
            lo, hi = 128 * c, min(128 * (c + 1), D)
            tmp_qkv[c, :, 0:hi - lo] = wt[:, lo:hi]
        for t in range(3):
            for d in range(DH):
                rows = [tmp_qkv[c, pl.ds(t * D + d, H, stride=DH), 0:min(128, D - 128 * c)] for c in range(4)]
                blk = jnp.concatenate(rows, axis=1)
                wqkvT[pl.ds((t * D + d * H) // 2, H // 2), :] = _pack(blk.astype(bf16))

    def prep_wo():
        wof = _unpack(wo_v[...]).astype(f32)
        for c in range(4):
            lo, hi = 128 * c, min(128 * (c + 1), D)
            tmp_o[c, :, 0:hi - lo] = wof[:, lo:hi]
        blks = []
        for d in range(DH):
            rows = [tmp_o[c, pl.ds(d, H, stride=DH), 0:min(128, D - 128 * c)] for c in range(4)]
            blks.append(jnp.concatenate(rows, axis=1))
        woT[...] = _pack(jnp.concatenate(blks, axis=0).T.astype(bf16))
        kT[:, 0:PAD] = jnp.zeros((D // 2, PAD), u32)
        vT[:, 0:PAD] = jnp.zeros((D // 2, PAD), u32)

    def qkv_proj(j):
        qkv = jnp.dot(_unpack(wqkvT[...]), _unpack(xnT[:, _cols(j)]), preferred_element_type=f32)
        kT[:, _cols(j, PAD)] = _pack(qkv[D:2 * D].astype(bf16))
        vT[:, _cols(j, PAD)] = _pack(qkv[2 * D:3 * D].astype(bf16))
        return qkv[0:D]

    def mix2(j):
        y = jnp.dot(_unpack(u_v[...]), _unpack(w2_v[j]), preferred_element_type=f32)
        return y + b2_v[_cols(j)].astype(f32)[None, :]

    def attention(j, q):
        win = slice(j * TB, (j + 1) * TB + PAD)
        kw = kT[:, win]
        vw = vT[:, win]
        pos = j * TB + jax.lax.broadcasted_iota(jnp.int32, (H, TB), 1)
        scale = DH ** -0.5
        logits = []
        for w in range(W):
            ks = kw if w == 0 else pltpu.roll(kw, DIL * w, 1)
            ks = _unpack(ks[:, PAD:]).astype(f32)
            lg = (q * ks).reshape(DH, H, TB).sum(axis=0) * scale
            if j * TB < DIL * w:
                lg = jnp.where(pos >= DIL * w, lg, -1e9)
            logits.append(lg)
        mx = functools.reduce(jnp.maximum, logits)
        es = [jnp.exp(l - mx) for l in logits]
        inv = 1.0 / functools.reduce(jnp.add, es)
        o = None
        for w in range(W):
            vs = vw if w == 0 else pltpu.roll(vw, DIL * w, 1)
            vs = _unpack(vs[:, PAD:]).astype(f32).reshape(DH, H, TB)
            term = vs * (es[w] * inv)[None]
            o = term if o is None else o + term
        return o.reshape(D, TB).astype(bf16)

    def finish(j, y, oT):
        attnT = jnp.dot(_unpack(woT[...]), oT, preferred_element_type=f32)
        res = y + attnT + _unpack(x_v[:, _cols(j)]).astype(f32)
        if j < NT - 1:
            out_v[j] = res.astype(bf16)
            out_copy(j).start()
        else:
            for p in range(NLAST):
                out_v[j, p * RL:(p + 1) * RL, :] = res[p * RL:(p + 1) * RL].astype(bf16)
                last_copies[p].start()

    for n in _ORDER:
        dma[n].start()
    wait("x0")
    layer_norm(0)
    fence = pltpu.make_async_copy(xnT.at[pl.ds(D // 2 - 8, 8), pl.ds(128, 128)], fence_v, isem.at[_SEM["fence"]])
    fence.start()
    wait("b1", "w1_0a")
    acc_v[:, 0:F0] = mix1(0, 0, F0) + b1_v[0:F0].astype(f32)[None, :]
    wait("w1_0b", "x1")
    fence.wait()
    acc_v[:, F0:F] = mix1(0, F0, F) + b1_v[F0:F].astype(f32)[None, :]
    layer_norm(1)

    def sweep(i, carry):
        pltpu.make_async_copy(w1_hbm.at[_w1_rows(i), :], w1_v.at[_w1_rows(i), :], isem.at[NT + i]).wait()
        pltpu.make_async_copy(x_hbm.at[:, _cols(i + 1)], x_v.at[:, _cols(i + 1)], isem.at[i + 1]).wait()
        acc_v[...] = acc_v[...] + mix1(i)
        layer_norm(i + 1)
        return carry

    jax.lax.fori_loop(1, NT - 3, sweep, 0)

    wait("w1_5", "x6")
    p5 = mix1(NT - 3)
    layer_norm(NT - 2)
    wait("x7", "w1_6", "w1_7", "wqkv", "wo")
    p6 = mix1(NT - 2)
    layer_norm(NT - 1)
    p7 = mix1(NT - 1)
    u_v[...] = _pack(_gelu(acc_v[...] + p5 + p6 + p7).astype(bf16))
    prep_wqkv()
    prep_wo()
    q = qkv_proj(0)

    for j in range(NT):
        if j == 0:
            wait("b2", "w2_0", "w2_1")
        if j == 2:
            wait("w2_2", "w2_3", "w2_4", "w2_5", "w2_6", "w2_7")
        y = mix2(j)
        oT = attention(j, q)
        if j + 1 < NT:
            q = qkv_proj(j + 1)
        finish(j, y, oT)

    for j in range(NT - 1):
        out_copy(j).wait()
    for c in last_copies:
        c.wait()


@jax.jit
def pallas_parallel_sum__sliding_local_dilated__mixer_token_mlp__prompt_kernel(
    A_x: jax.Array,
    A_wqkv: jax.Array,
    A_wo: jax.Array,
    B_x: jax.Array,
    B_w1: jax.Array,
    B_b1: jax.Array,
    B_w2: jax.Array,
    B_b2: jax.Array,
):
    del B_x
    xT = A_x.reshape(S, D).T
    hbm = pl.BlockSpec(memory_space=pltpu.HBM)
    outT = pl.pallas_call(
        _kernel,
        out_shape=jax.ShapeDtypeStruct((D, S), bf16),
        in_specs=[hbm] * 7,
        out_specs=hbm,
        scratch_shapes=[
            pltpu.VMEM((F,), bf16),
            pltpu.VMEM((S,), bf16),
            pltpu.VMEM((D // 2, S), u32),
            pltpu.VMEM((D // 2, 3 * D), u32),
            pltpu.VMEM((D // 2, D), u32),
            pltpu.VMEM((S // 2, F), u32),
            pltpu.VMEM((NT, F // 2, TB), u32),
            pltpu.VMEM((D // 2, S), u32),
            pltpu.VMEM((3 * D // 2, D), u32),
            pltpu.VMEM((D // 2, D), u32),
            pltpu.VMEM((D, F), f32),
            pltpu.VMEM((D // 2, F), u32),
            pltpu.VMEM((D // 2, S + PAD), u32),
            pltpu.VMEM((D // 2, S + PAD), u32),
            pltpu.VMEM((4, 3 * D, 128), f32),
            pltpu.VMEM((4, D, 128), f32),
            pltpu.VMEM((NT, D, TB), bf16),
            pltpu.VMEM((8, 128), u32),
            pltpu.SemaphoreType.DMA((3 * NT + 6,)),
            pltpu.SemaphoreType.DMA((NT - 1 + NLAST,)),
        ],
        compiler_params=pltpu.CompilerParams(
            vmem_limit_bytes=100 * 1024 * 1024, disable_bounds_checks=True, disable_semaphore_checks=True,
            flags={"XLA_TPU_RESCHEDULE_DMA_DONES": True}),
        name="fused_attn_mixer",
    )(xT, A_wqkv, A_wo, B_w1, B_b1, B_w2, B_b2)
    return outT.T.reshape(1, S, D)
```
